```python
import os as _os
_os.environ.setdefault("JAX_PLATFORMS", "cpu")
import jax
import jax.numpy as jnp

def _softmax(x, axis=-1):
    return jax.nn.softmax(x, axis=axis)
def _gelu(x):
    return jax.nn.gelu(x, approximate=True)
def _silu(x):
    return jax.nn.silu(x)
def _sigmoid(x):
    return jax.nn.sigmoid(x)
def _layernorm(x, axis=-1, eps=1e-5):
    m = jnp.mean(x, axis=axis, keepdims=True)
    v = jnp.var(x, axis=axis, keepdims=True)
    return (x - m) / jnp.sqrt(v + eps)
def _scatter_add(tgt, idx, src, axis=0):
    return tgt.at[idx].add(src)
def _segment_sum(src, seg, n):
    return jax.ops.segment_sum(src, seg, n)
class _Rng:
    def __init__(self, key):
        self._k = key
    def _next(self):
        self._k, sub = jax.random.split(self._k)
        return sub
    def normal(self, shape):
        return jax.random.normal(self._next(), shape, dtype=jnp.bfloat16)
    def randint(self, lo, hi, shape):
        return jax.random.randint(self._next(), shape, lo, hi, dtype=jnp.int32)
    def uniform(self, shape, lo=0.0, hi=1.0):
        return jax.random.uniform(self._next(), shape, jnp.bfloat16, lo, hi)
    def permutation(self, n):
        return jax.random.permutation(self._next(), n)


kernel_name = 'standalone__mha_softmax__prompt'

def setup_inputs():
    _rng = _Rng(jax.random.key(int.from_bytes(__import__("os").urandom(4), "little")))
    _w = (lambda a: (lambda t: t.astype(jnp.bfloat16) if jnp.issubdtype(t.dtype, jnp.floating) else t)(jnp.asarray(a)))
    B, H, Sq, Sk, D = 1, 32, 2048, 2048, 192
    return {
        "q": _w((lambda *s: _rng.normal(s) * 0.4)(B, H, Sq, D)),
        "k": _w((lambda *s: _rng.normal(s) * 0.4)(B, H, Sk, D)),
        "v": _w((lambda *s: _rng.normal(s) * 0.05)(B, H, Sk, D)),
    }

def reference(q, k, v):
    scale = q.shape[-1] ** -0.5
    scores = jnp.einsum("bhqd,bhkd->bhqk", q, k) * scale
    p = _softmax(scores, axis=-1)
    return jnp.einsum("bhqk,bhkd->bhqd", p, v)
```

```python
import functools, math
import jax, jax.numpy as jnp
import jax.experimental.pallas as pl
import jax.experimental.pallas.tpu as pltpu

F32 = jnp.float32
BF16 = jnp.bfloat16
U32 = jnp.uint32

def make(R=256, lag=2, kg=4, tok=2, tail_tok=3, NB=4, W=128, vscr=True, kpipe=True, kpieces=8, kstart=8):
    def prep_piece(kT_ref, L_scr, slot, c0, c1, HS, tokv=None):
        ka = kT_ref[:, c0:c1]; kb = kT_ref[:, HS + c0:HS + c1]
        d1 = ka[64:128].astype(F32) - kb[64:128].astype(F32)
        d2 = kb[0:64].astype(F32) - ka[0:64].astype(F32)
        d1 = d1.astype(BF16); d2 = d2.astype(BF16)
        r = slice(c0 // 2, c1 // 2)
        L_scr[slot, 0, r, :] = pltpu.bitcast(jnp.concatenate([ka[0:64], kb[64:128]], axis=0).T, U32)
        L_scr[slot, 1, r, :] = pltpu.bitcast(jnp.concatenate([d1, ka[128:192]], axis=0).T, U32)
        L_scr[slot, 2, r, :] = pltpu.bitcast(jnp.concatenate([d2, kb[128:192]], axis=0).T, U32)

    def kern(qT_ref, k0_ref, kT_ref, vT_ref, oT_ref, L_scr, S_scr, V_scr):
        D, S = qT_ref.shape
        HS = S // 2
        c = (D ** -0.5) * math.log2(math.e)
        h = pl.program_id(0)
        par = h % 2
        if kpipe:
            @pl.when(h == 0)
            def _():
                prep_piece(k0_ref, L_scr, 0, 0, HS, HS)
        else:
            prep_piece(kT_ref, L_scr, par, 0, HS, HS)
        nt = S // W
        nch = HS // R
        nkt = S // 128
        npv = nkt // kg
        st = [dict(m=None, l=None, acc=None) for _ in range(nt)]
        toks = []
        qtoks = []

        if vscr:
            for j in range(nkt):
                V_scr[par, j] = pltpu.bitcast(vT_ref[:, j*128:(j+1)*128], U32)

        def qk(n, ci):
            t = st[n]
            if ci == 0:
                t['q'] = qT_ref[:, n*W:(n+1)*W]
            q = t['q']
            w12 = q[0:128]; w23 = q[64:192]
            w13 = jnp.concatenate([q[0:64], q[128:192]], axis=0)
            r = slice(ci*R//2, (ci+1)*R//2)
            ld = lambda i: pltpu.bitcast(L_scr[par, i, r, :], BF16)
            p3 = jnp.dot(ld(0), w12, preferred_element_type=F32)
            p1 = jnp.dot(ld(1), w23, preferred_element_type=F32)
            p2 = jnp.dot(ld(2), w13, preferred_element_type=F32)
            sa = p1 + p3; sb = p2 + p3
            qtoks.append(sa[0:8])
            S_scr[par, n % NB, ci*R:(ci+1)*R, :] = sa
            S_scr[par, n % NB, HS+ci*R:HS+(ci+1)*R, :] = sb
            mm = jnp.maximum(sa, sb).reshape(R // 8, 8, W).max(axis=0)
            t['m'] = mm if t['m'] is None else jnp.maximum(t['m'], mm)
            if ci == nch - 1:
                t['m'] = jnp.broadcast_to(jnp.max(t['m'], axis=0, keepdims=True), (8, W))

        def pv(n, j, tk):
            t = st[n]
            ks = slice(j*kg*128, (j+1)*kg*128)
            m = t['m']
            x = None
            if tk and len(toks) >= tk:
                x = toks[-tk]
            elif tk and len(toks) >= 1:
                x = qtoks[-2]
            if x is not None:
                m = jnp.where(x > jnp.inf, x, m)
            s = S_scr[par, n % NB, ks, :]
            s = s.reshape(kg * 16, 8, W)
            p = jnp.exp2((s - m[None]) * c)
            ls = p.sum(axis=0)
            p = p.reshape(kg * 128, W)
            t['l'] = ls if t['l'] is None else t['l'] + ls
            if vscr:
                vt = jnp.concatenate([pltpu.bitcast(V_scr[par, jj], BF16) for jj in range(j*kg, (j+1)*kg)], axis=1)
            else:
                vt = vT_ref[:, ks]
            o = jnp.dot(vt, p.astype(BF16), preferred_element_type=F32)
            toks.append(o[0:8])
            t['acc'] = o if t['acc'] is None else t['acc'] + o
            if j == npv - 1:
                l = jnp.sum(t['l'], axis=0, keepdims=True)
                oT_ref[:, n*W:(n+1)*W] = (t['acc'] * (1.0 / l)).astype(oT_ref.dtype)
                st[n] = None

        qks = [(n, ci) for n in range(nt) for ci in range(nch)]
        pvs = [(n, j) for n in range(nt) for j in range(npv)]
        lead = nch + lag
        qi = 0
        kp = 0
        pw = HS // kpieces
        for pi, (n, j) in enumerate(pvs):
            target = min(len(qks), lead + (pi * nch) // npv)
            while qi < target:
                qk(*qks[qi]); qi += 1
            pv(n, j, tok if qi < len(qks) else tail_tok)
            if kpipe and pi >= kstart and (pi - kstart) % 4 == 0 and kp < kpieces:
                prep_piece(kT_ref, L_scr, 1 - par, kp * pw, (kp + 1) * pw, HS)
                kp += 1
        assert qi == len(qks)

    @jax.jit
    def f(q, k, v):
        B, H, S, D = q.shape
        NH = B * H
        qT = jnp.swapaxes(q, 2, 3).reshape(NH, D, S)
        kT = jnp.swapaxes(k, 2, 3).reshape(NH, D, S)
        vT = jnp.swapaxes(v, 2, 3).reshape(NH, D, S)
        kmap = (lambda h: (jnp.minimum(h + 1, NH - 1), 0, 0)) if kpipe else (lambda h: (h, 0, 0))
        oT = pl.pallas_call(
            kern,
            grid=(NH,),
            in_specs=[pl.BlockSpec((None, D, S), lambda h: (h, 0, 0)),
                      pl.BlockSpec((None, D, S), lambda h: (0, 0, 0)),
                      pl.BlockSpec((None, D, S), kmap),
                      pl.BlockSpec((None, D, S), lambda h: (h, 0, 0))],
            out_specs=pl.BlockSpec((None, D, S), lambda h: (h, 0, 0)),
            out_shape=jax.ShapeDtypeStruct((NH, D, S), q.dtype),
            scratch_shapes=[pltpu.VMEM((2, 3, S // 4, 128), U32), pltpu.VMEM((2, NB, S, W), F32),
                            pltpu.VMEM((2, S // 128, D // 2, 128), U32)],
            compiler_params=pltpu.CompilerParams(dimension_semantics=("arbitrary",),
                                                 vmem_limit_bytes=100*1024*1024),
        )(qT, kT, kT, vT)
        return jnp.swapaxes(oT.reshape(B, H, D, S), 2, 3)
    return f


_impl = make()


@jax.jit
def pallas_standalone__mha_softmax__prompt_kernel(q: jax.Array, k: jax.Array, v: jax.Array):
    return _impl(q, k, v)
```

```python
import bisect
import math
import jax, jax.numpy as jnp
import jax.experimental.pallas as pl
import jax.experimental.pallas.tpu as pltpu

F32 = jnp.float32
BF16 = jnp.bfloat16
U32 = jnp.uint32


def plan(CH, nt, HS, G):
    sizes = [CH] * (HS // CH) + ([HS % CH] if HS % CH else [])
    nch = len(sizes)
    NQ = nt * nch
    NM = (nt // 2) * 56
    return sizes, nch, NQ, NM


def make(CH=96, mQL=150, mLP=150, mPM=500, tail=250, NB=4, NBB=4, kpieces=8, kt0=600, kt1=12000, vt0=13000, vt1=21000,
         QW=1024, verbose=False):
    W = 128; G = 96
    NSTATE = 8
    KEYS = ('m', 'l', 'M')
    S = 2048; HS = S // 2; nt = S // W; nT = nt // 2; nj = HS // 128
    sizes, nch, NQ, NM = plan(CH, nt, HS, G)
    offs = [sum(sizes[:i]) for i in range(nch)]
    TOT = (3 * HS * nt + NM * G) // 4
    PER = TOT / nT
    NCL = 64

    lead_p = PER + mPM
    lead_l = lead_p + PER + mLP
    lead_q = lead_l + PER / 2 + mQL
    span = TOT - tail
    LP_ = int(math.ceil(lead_p / PER * NCL))
    LL_ = int(math.ceil(lead_l / PER * NCL))
    LQ_ = int(math.ceil(lead_q / (PER / 2) * nch)) + 1

    order = []
    load = [0, 0, 0, 0]
    mi = 0
    rows_done = 0
    def put(n):
        u = min(range(4), key=lambda u: load[u]); s = load[u]; load[u] += n; return s
    for k in range(NQ):
        sz = sizes[(k + LQ_) % nch]
        s = max(put(sz) for _ in range(3))
        order.append(('q', k, s, sz))
        rows_done += sz
        while mi < NM and min(load) + G // 2 <= sorted(load)[1]:
            order.append(('m', mi, put(G), G)); mi += 1
        target = rows_done * NM / (nt * HS)
        while mi + 4 <= target + 2 and mi + 4 <= NM:
            for _ in range(4):
                order.append(('m', mi, put(G), G)); mi += 1
    while mi < NM:
        order.append(('m', mi, put(G), G)); mi += 1
    cands = sorted((s + 8 * i, pos, i) for pos, (kd, idx, s, sz) in enumerate(order) for i in range(sz // 8))
    ctimes = [c[0] for c in cands]
    def pick(t):
        i = min(bisect.bisect_left(ctimes, t), len(cands) - 1)
        best = min(cands[i:i + 4], key=lambda c: c[1])
        return best[1], best[2]
    tasks = []
    NC = NCL * nT
    for i in range(NC):
        tasks.append(((i + 0.25) * span / NC, 'l', i + LL_))
        tasks.append(((i + 0.75) * span / NC, 'p', i + LP_))
    for i in range(kpieces):
        tasks.append((kt0 + i * (kt1 - kt0) / kpieces, 'k', i))
    nv = 6
    for i in range(nj * nv):
        tasks.append((vt0 + i * (vt1 - vt0) / (nj * nv), 'v', i))
    tasks.sort()
    after = [[] for _ in order]
    cur = 0
    for t, kd, idx in tasks:
        pos, vr = pick(t)
        cur = max(cur, pos)
        after[cur].append((kd, idx, pos, vr))
    if verbose:
        print("TOT", TOT, "LQ", LQ_, "LL", LL_, "LP", LP_, "load", load, "nch", nch)
        print("".join(o[0] for o in order)[:400])

    def kern(qT_ref, qn_ref, k0_ref, kn_ref, v0_ref, vn_ref, oT_ref, z_ref, Lc_scr, Ln_scr, Ac_scr, An_scr, st_scr, *rest):
        S_refs = rest[:NB]; B_refs = rest[NB:NB + NBB]
        D = qT_ref.shape[0]
        HD = D // 2
        c = (D ** -0.5) * math.log2(math.e)
        h = pl.program_id(0)
        BROWS = 7 * (HS // 2)
        ASZ = 7 * nj * (HD // 2)

        def body(prologue):
            if prologue:
                q_next, k_next, v_next = qT_ref, k0_ref, v0_ref
            else:
                q_next, k_next, v_next = qn_ref, kn_ref, vn_ref
            z = z_ref[0]
            zb = pl.multiple_of(z * 8, 8)
            LSZ = HS // 2
            s_fence = pl.ds(pl.multiple_of(2 * S + z * 8, 8), 8)
            b_fence = pl.ds(pl.multiple_of(BROWS + z * 8, 8), 8)
            st = [dict() for _ in range(nt + NSTATE)]
            cst = [dict() for _ in range(nT)]
            res = {}
            done = dict(k=0, q=set(), l=set(), p=set())

            def gate(x, *ms):
                if x is None: return ms
                cnd = x > jnp.inf
                return tuple(jnp.where(cnd, x, m) for m in ms)

            def kprep(c0, c1):
                ka = k_next[:, c0:c1]; kb = k_next[:, HS + c0:HS + c1]
                d1 = (ka[64:128].astype(F32) - kb[64:128].astype(F32)).astype(BF16)
                d2 = (kb[0:64].astype(F32) - ka[0:64].astype(F32)).astype(BF16)
                rr = lambda i: pl.ds(zb + i * LSZ + c0 // 2, (c1 - c0) // 2)
                Ln_scr[rr(0), :] = pltpu.bitcast(jnp.concatenate([ka[0:64], kb[64:128]], axis=0).T, U32)
                Ln_scr[rr(1), :] = pltpu.bitcast(jnp.concatenate([d1, ka[128:192]], axis=0).T, U32)
                Ln_scr[rr(2), :] = pltpu.bitcast(jnp.concatenate([d2, kb[128:192]], axis=0).T, U32)

            def vprep(idx, x):
                j, r = divmod(idx, nv)
                def ldv(r0, c0):
                    u = pltpu.bitcast(v_next[r0 + 16*r:r0 + 16*r + 16, c0:c0 + 128], U32)
                    if x is not None:
                        u = jnp.where(x > jnp.inf, pltpu.bitcast(x, U32), u)
                    return u
                u11 = ldv(0, j*128); u21 = ldv(HD, j*128); u12 = ldv(0, HS + j*128); u22 = ldv(HD, HS + j*128)
                def unp(u):
                    return [pltpu.unpack_elementwise(u, index=i, packed_dtype=BF16, unpacked_dtype=F32) for i in range(2)]
                f11, f12, f21, f22 = unp(u11), unp(u12), unp(u21), unp(u22)
                pk = lambda a, b, sg: pltpu.pack_elementwise(
                    [a[i] + b[i] if sg > 0 else a[i] - b[i] for i in range(2)], packed_dtype=BF16).astype(U32)
                As = [pk(f11, f22, 1), pk(f21, f22, 1), u11, u22, pk(f11, f12, 1), pk(f21, f11, -1), pk(f12, f22, -1)]
                for i in range(7):
                    An_scr[pl.ds(zb + (i*nj + j)*(HD//2) + 8*r, 8), :] = As[i]

            def qk(n, ci):
                t = st[n]
                nxt = n >= nt
                if nxt: assert prologue or done['k'] == kpieces
                if 'q' not in t:
                    t['q'] = q_next[:, (n-nt)*W:(n-nt+1)*W] if nxt else qT_ref[:, n*W:(n+1)*W]
                q = t['q']
                w12 = q[0:128]; w23 = q[64:192]
                w13 = jnp.concatenate([q[0:64], q[128:192]], axis=0)
                r0 = offs[ci]; R = sizes[ci]
                Lr = Ln_scr if nxt else Lc_scr
                ld = lambda i: pltpu.bitcast(Lr[pl.ds(zb + i * LSZ + r0 // 2, R // 2), :], BF16)
                p3 = jnp.dot(ld(0), w12, preferred_element_type=F32)
                p1 = jnp.dot(ld(1), w23, preferred_element_type=F32)
                p2 = jnp.dot(ld(2), w13, preferred_element_type=F32)
                sa = (p1 + p3) * c; sb = (p2 + p3) * c
                Sr = S_refs[(n // 2) % NB]; o0 = (n % 2) * S
                Sr[o0+r0:o0+r0+R, :] = sa
                Sr[o0+HS+r0:o0+HS+r0+R, :] = sb
                mm = jnp.maximum(sa, sb).reshape(R // 8, 8, W).max(axis=0)
                t['m'] = jnp.maximum(t['m'], mm) if 'm' in t else mm
                if ci == nch - 1:
                    t['m'] = jnp.broadcast_to(jnp.max(t['m'], axis=0, keepdims=True), (8, W))
                    Sr[s_fence, :] = t['m']
                    done['q'].add(n)
                return sa

            def lcl(idx, x):
                n, u = divmod(idx, NCL // 2)
                assert n in done['q'], ("l before q", n)
                t = st[n]
                rows = 64
                r0 = (n % 2) * S + u * rows
                s = S_refs[(n // 2) % NB][r0:r0 + rows, :].reshape(rows // 8, 8, W)
                m, = gate(x, t['m'])
                p = jnp.exp2(s - m[None])
                xs = [p[i] for i in range(rows // 8)]
                while len(xs) > 1:
                    xs = [xs[i] + xs[i+1] for i in range(0, len(xs), 2)]
                t['l'] = t['l'] + xs[0] if 'l' in t else xs[0]
                if u == NCL // 2 - 1:
                    l = jnp.sum(t['l'], axis=0, keepdims=True)
                    t['M'] = t['m'] + jnp.broadcast_to(jnp.log2(l), (8, W))
                    del t['m'], t['l']

            def pcl(idx, x):
                T, k = divmod(idx, NCL)
                n1, n2 = 2*T, 2*T + 1
                Br = B_refs[T % NBB]
                r0 = k * 16
                def P(n, M, base, odd):
                    s = S_refs[T % NB][pl.ds((n % 2) * S + base + r0 + odd, 8, stride=2), :]
                    return jnp.exp2(s - M)
                M1, M2 = gate(x, st[n1]['M'], st[n2]['M'])
                Bs = []
                for odd in range(2):
                    b11 = P(n1, M1, 0, odd); b21 = P(n1, M1, HS, odd); b12 = P(n2, M2, 0, odd); b22 = P(n2, M2, HS, odd)
                    Bs.append([b11 + b22, b11, b12 - b22, b21 - b11, b22, b11 + b12, b21 + b22])
                for i in range(7):
                    off = i * (HS // 2) + r0 // 2
                    Br[off:off + 8, :] = pltpu.pack_elementwise([Bs[0][i], Bs[1][i]], packed_dtype=BF16).astype(U32)
                if k == NCL - 1:
                    Br[b_fence, :] = pltpu.bitcast(st[n1]['M'], U32)
                    del st[n1]['M'], st[n2]['M']
                    done['p'].add(T)

            comb = {0: [('11', 1), ('22', 1)], 1: [('21', 1), ('22', -1)], 2: [('12', 1), ('22', 1)],
                    3: [('11', 1), ('21', 1)], 4: [('11', -1), ('12', 1)], 5: [('22', 1)], 6: [('11', 1)]}
            def mgroup(g):
                T, r = divmod(g, 56); i, j = divmod(r, 8)
                assert T in done['p'], ("m before p", T)
                a = pltpu.bitcast(Ac_scr[pl.ds(zb + (i*nj + j)*(HD//2), HD//2), :], BF16)
                b = pltpu.bitcast(B_refs[T % NBB][i*(HS//2) + j*64:i*(HS//2) + (j+1)*64, :], BF16)
                oj = jnp.dot(a, b, preferred_element_type=F32)
                cs = cst[T]
                cs['o'] = oj if j == 0 else cs['o'] + oj
                if j == nj - 1:
                    o = cs['o']
                    for name, sg in comb[i]:
                        if name not in cs:
                            cs[name] = o if sg > 0 else -o
                        else:
                            cs[name] = cs[name] + o if sg > 0 else cs[name] - o
                    if i == 6:
                        q0 = 2*T*W
                        oT_ref[0:HD, q0:q0+W] = cs['11'].astype(oT_ref.dtype)
                        oT_ref[0:HD, q0+W:q0+2*W] = cs['12'].astype(oT_ref.dtype)
                        oT_ref[HD:D, q0:q0+W] = cs['21'].astype(oT_ref.dtype)
                        oT_ref[HD:D, q0+W:q0+2*W] = cs['22'].astype(oT_ref.dtype)
                return oj

            def live_keys(n):
                T = n // 2
                ks = []
                qdone = max(0, min(nch, LQ_ - n * nch))
                ldone = max(0, min(NCL // 2, LL_ - n * (NCL // 2)))
                pdone = max(0, min(NCL, LP_ - T * NCL))
                if qdone > 0 and ldone < NCL // 2: ks.append('m')
                if 0 < ldone < NCL // 2: ks.append('l')
                if ldone == NCL // 2 and pdone < NCL: ks.append('M')
                return ks

            if prologue:
                kprep(0, HS)
                for i in range(nj * nv): vprep(i, None)
            else:
                Lc_scr[pl.ds(zb, 3 * LSZ), :] = Ln_scr[pl.ds(zb, 3 * LSZ), :]
                Ac_scr[pl.ds(zb, ASZ), :] = An_scr[pl.ds(zb, ASZ), :]
                for n in range(NSTATE):
                    for key in live_keys(n):
                        st[n][key] = st_scr[n * 3 + KEYS.index(key)]
                    if LQ_ >= (n + 1) * nch: done['q'].add(n)
                    if LP_ >= (n // 2 + 1) * NCL: done['p'].add(n // 2)
            pw = HS // kpieces
            last_q = None
            for pos, (kd, idx, s0, sz) in enumerate(order):
                if kd == 'q':
                    n, ci = divmod(idx + LQ_, nch)
                    if not prologue or n >= nt:
                        res[pos] = qk(n, ci); last_q = pos
                elif not prologue:
                    res[pos] = mgroup(idx)
                for tk, ti, tpos, vr in after[pos]:
                    if prologue:
                        if tk in 'kv' or ti < NC: continue
                        if tpos not in res:
                            tpos = last_q; vr = min(vr, res[tpos].shape[0] // 8 - 1)
                    x = res[tpos][8*vr:8*vr+8]
                    if tk == 'l': lcl(ti, x)
                    elif tk == 'p': pcl(ti, x)
                    elif tk == 'v': vprep(ti, x)
                    else:
                        kprep(ti * pw, (ti + 1) * pw); done['k'] += 1
            for n in range(NSTATE):
                keys = [k for k in st[nt + n] if k != 'q']
                assert sorted(keys) == sorted(live_keys(n)), (n, keys, live_keys(n))
                for key in keys:
                    st_scr[n * 3 + KEYS.index(key)] = st[nt + n][key]

        @pl.when(h == 0)
        def _():
            z_ref[0] = 0
            body(True)
        body(False)

    @jax.jit
    def f(q, k, v):
        B, H, S_, D = q.shape
        NH = B * H
        qT = jnp.swapaxes(q, 2, 3).reshape(NH, D, S)
        kT = jnp.swapaxes(k, 2, 3).reshape(NH, D, S)
        vT = jnp.swapaxes(v, 2, 3).reshape(NH, D, S)
        cur = lambda h: (h, 0, 0)
        nxt = lambda h: (jnp.minimum(h + 1, NH - 1), 0, 0)
        first = lambda h: (0, 0, 0)
        oT = pl.pallas_call(
            kern,
            grid=(NH,),
            in_specs=[pl.BlockSpec((None, D, S), cur), pl.BlockSpec((None, D, QW), nxt),
                      pl.BlockSpec((None, D, S), first), pl.BlockSpec((None, D, S), nxt),
                      pl.BlockSpec((None, D, S), first), pl.BlockSpec((None, D, S), nxt)],
            out_specs=pl.BlockSpec((None, D, S), cur),
            out_shape=jax.ShapeDtypeStruct((NH, D, S), q.dtype),
            scratch_shapes=[pltpu.SMEM((1,), jnp.int32), pltpu.VMEM((3 * (S // 4), 128), U32), pltpu.VMEM((3 * (S // 4), 128), U32),
                            pltpu.VMEM((7 * (S // 256) * (D // 4), 128), U32),
                            pltpu.VMEM((7 * (S // 256) * (D // 4), 128), U32),
                            pltpu.VMEM((NSTATE * 3, 8, 128), F32)]
                           + [pltpu.VMEM((2 * S + 8, W), F32) for _ in range(NB)]
                           + [pltpu.VMEM((7 * (S // 4) + 8, 128), U32) for _ in range(NBB)],
            compiler_params=pltpu.CompilerParams(dimension_semantics=("arbitrary",),
                                                 vmem_limit_bytes=100*1024*1024),
        )(qT, qT, kT, kT, vT, vT)
        return jnp.swapaxes(oT.reshape(B, H, D, S), 2, 3)
    return f


_impl = make(CH=192)


@jax.jit
def pallas_standalone__mha_softmax__prompt_kernel(q: jax.Array, k: jax.Array, v: jax.Array):
    return _impl(q, k, v)
```

```python
import bisect
import math
import jax, jax.numpy as jnp
import jax.experimental.pallas as pl
import jax.experimental.pallas.tpu as pltpu

F32 = jnp.float32
BF16 = jnp.bfloat16
U32 = jnp.uint32


def make(N=4, CH=208, mQL=150, mLP=150, mPM=500, tail=250, NB=16, NBB=4, kpieces=8, kt0=600, kt1=6000,
         vt0=6500, vt1=21000, mearly=0, GV=4, espan=300, psq=1.0, csz=4, last=True, verbose=False):
    W = 128; G = 96
    S = 2048; HS = S // 2; nt = S // W; nT = nt // N
    KB = S // N; ng = KB // 128
    NSTATE = 12
    KEYS = ('m', 'e', 'M', 'l')
    lam = [1.0 / math.tan(math.pi * (i + 1) / (N + 1)) for i in range(N)]
    sgn = lambda i, j: 1.0 if (i + j) % 2 == 1 else -1.0
    pairs = [(i, j) for i in range(N) for j in range(i + 1, N)]
    prods = []
    for i in range(N):
        for j in range(i + 1, N):
            prods += [('s', i, j), ('x', i, j), ('y', i, j)]
        prods += [('e', i, i), ('f', i, i)]
    NP = len(prods); pidx = {p: k for k, p in enumerate(prods)}
    if N == 2:
        subs = [[('d', 0, 1), ('p', 0, 1)]] if csz == 8 else [[('d', 0, 1)], [('p', 0, 1)]]
    else:
        seq = [('d', 0, 2), ('p', 0, 2), ('d', 1, 3), ('p', 1, 3), ('p', 0, 1), ('p', 2, 3), ('p', 0, 3), ('p', 1, 2)]
        subs = [[x] for x in seq] if csz == 4 else [seq[0:2], seq[2:4], seq[4:6], seq[6:8]]
    nsub = len(subs)
    sizes = [CH] * (HS // CH) + ([HS % CH] if HS % CH else [])
    nch = len(sizes); offs = [sum(sizes[:i]) for i in range(nch)]
    NQ = nt * nch; GPT = NP * ng; NM = nT * GPT
    TOT = (3 * HS * nt + NM * G) // 4
    PER = TOT / nT
    NCL = (KB // 16) * nsub
    ngv = [-(-(sz // 8) // GV) for sz in sizes]
    goff = [sum(ngv[:i]) for i in range(nch)]; NGV = sum(ngv)
    NEC = -(-NGV // 8)
    lead_p = PER + mPM
    lead_q = lead_p + PER + mLP + espan + mQL
    span = TOT - tail
    LP_ = int(math.ceil(lead_p / PER * NCL / nsub)) * nsub
    LQ_ = int(math.ceil(lead_q / (PER / N) * nch)) + 1

    order = []
    load = [0, 0, 0, 0]
    mi = 0; rows_done = 0
    def put(n):
        u = min(range(4), key=lambda u: load[u]); s = load[u]; load[u] += n; return s
    for k in range(NQ):
        sz = sizes[(k + LQ_) % nch]
        s = max(put(sz) for _ in range(3))
        order.append(('q', k, s, sz))
        rows_done += sz
        while mi < NM and min(load) + G // 2 <= sorted(load)[1]:
            order.append(('m', mi, put(G), G)); mi += 1
        target = rows_done * NM / (nt * HS - mearly)
        while mi + 4 <= target + 2 and mi + 4 <= NM:
            for _ in range(4):
                order.append(('m', mi, put(G), G)); mi += 1
    while mi < NM:
        order.append(('m', mi, put(G), G)); mi += 1
    cands = sorted((s + 8 * i, pos, i) for pos, (kd, idx, s, sz) in enumerate(order) for i in range(sz // 8))
    ctimes = [c[0] for c in cands]
    def pick(t):
        i = min(bisect.bisect_left(ctimes, t), len(cands) - 1)
        best = min(cands[i:i + 4], key=lambda c: c[1])
        return best[1], best[2]
    tasks = []
    NC = NCL * nT
    for i in range(NC):
        tasks.append((((i // nsub) * nsub + 0.5 + (i % nsub) * psq) * span / NC, 'p', i + LP_))
    LE_ = None
    for kd, idx, s0, sz in order:
        if kd == 'q' and (idx + LQ_) % nch == nch - 1:
            n = (idx + LQ_) // nch
            for u in range(NEC):
                t = s0 + sz + mQL + u * espan / NEC
                if t >= span: t -= span; n_ = n - nt
                else: n_ = n
                tasks.append((t, 'e', n_ * NEC + u))
    LE_ = min(ti for _, kd, ti in tasks if kd == 'e')
    for i in range(kpieces):
        tasks.append((kt0 + i * (kt1 - kt0) / kpieces, 'k', i))
    nv = 6
    vsub = len(pairs) + 1
    NV = ng * nv * vsub
    for i in range(NV):
        tasks.append((vt0 + i * (vt1 - vt0) / NV, 'v', i))
    tasks.sort()
    after = [[] for _ in order]
    cur = 0
    for t, kd, idx in tasks:
        pos, vr = pick(t)
        cur = max(cur, pos)
        after[cur].append((kd, idx, pos, vr))
    if verbose:
        print("TOT", TOT, "LQ", LQ_, "LE", LE_, "NEC", NEC, "LP", LP_, "load", load, "nch", nch, "NP", NP)

    def kern(q_next, k_next, v_next, oT_ref, z_ref, Lc_scr, Ln_scr, Ac_scr, An_scr, Qc_scr, G_scr, st_scr, *rest):
        S_refs = rest[:NB]; B_refs = rest[NB:NB + NBB]
        D = q_next.shape[0]
        HD = D // 2
        c = (D ** -0.5) * math.log2(math.e)
        h = pl.program_id(0)
        BROWS = NP * (KB // 2)
        ASZ = NP * ng * (HD // 2)

        def body(mode):
            prologue = mode == 'first'
            final = mode == 'last'
            z = z_ref[0]
            zb = pl.multiple_of(z * 8, 8)
            LSZ = HS // 2
            s_fence = pl.ds(pl.multiple_of(S + z * 8, 8), 8)
            b_fence = pl.ds(pl.multiple_of(BROWS + z * 8, 8), 8)
            st = [dict() for _ in range(nt + NSTATE)]
            cst = [dict() for _ in range(nT)]
            pst = {}
            res = {}
            done = dict(k=0, q=set(), p=set(), m=set())

            def gate(x, *ms):
                if x is None: return list(ms)
                cnd = x > jnp.inf
                return [jnp.where(cnd, x if m.dtype == F32 else pltpu.bitcast(x, m.dtype), m) for m in ms]

            def pack(a, b):
                return pltpu.pack_elementwise([a, b], packed_dtype=BF16).astype(U32)

            unp = lambda u: [pltpu.unpack_elementwise(u, index=i, packed_dtype=BF16, unpacked_dtype=F32) for i in range(2)]

            def kprep(c0, c1):
                def ldk(r0, cb):
                    return [t * c for t in unp(pltpu.bitcast(k_next[r0:r0 + 64, cb + c0:cb + c1], U32))]
                a1 = pack(*ldk(0, 0)); b2 = pack(*ldk(64, HS)); a3 = pack(*ldk(128, 0)); b3 = pack(*ldk(128, HS))
                d1 = pack(*[x - y for x, y in zip(ldk(64, 0), unp(b2))])
                d2 = pack(*[x - y for x, y in zip(ldk(0, HS), unp(a1))])
                rr = lambda i: pl.ds(zb + i * LSZ + c0 // 2, (c1 - c0) // 2)
                tr = lambda x, y: pltpu.bitcast(pltpu.bitcast(jnp.concatenate([x, y], axis=0), BF16).T, U32)
                Ln_scr[rr(0), :] = tr(a1, b2)
                Ln_scr[rr(1), :] = tr(d1, a3)
                Ln_scr[rr(2), :] = tr(d2, b3)

            def vprep(idx, x):
                pos_, sub = divmod(idx, vsub)
                j, r = divmod(pos_, nv)
                def ldv(half, kblk):
                    r0 = half * HD + 16 * r; c0 = kblk * KB + j * 128
                    return gate(x, pltpu.bitcast(v_next[r0:r0 + 16, c0:c0 + 128], U32))[0]
                def put_a(p, u):
                    An_scr[pl.ds(zb + (pidx[p] * ng + j) * (HD // 2) + 8 * r, 8), :] = u
                if sub == len(pairs):
                    for i in range(N):
                        u1 = ldv(0, i); a1 = unp(u1); a2 = unp(ldv(1, i))
                        put_a(('e', i, i), u1)
                        put_a(('f', i, i), pack(*[lam[i] * a1[t] + a2[t] for t in range(2)]))
                else:
                    i, jj = pairs[sub]
                    tau = sgn(i, jj); d = lam[i] - lam[jj]
                    a1i, a2i, a1j, a2j = unp(ldv(0, i)), unp(ldv(1, i)), unp(ldv(0, jj)), unp(ldv(1, jj))
                    xs, ys, ss = [], [], []
                    for t in range(2):
                        u = a1i[t] + a1j[t] if tau > 0 else a1i[t] - a1j[t]
                        w = a2i[t] + a2j[t] if tau > 0 else a2i[t] - a2j[t]
                        xn = u * (lam[jj] / d) + w * (1.0 / d)
                        xs.append(xn); ys.append(u + xn); ss.append(a1i[t] + xn)
                    put_a(('x', i, jj), pack(*xs)); put_a(('y', i, jj), pack(*ys)); put_a(('s', i, jj), pack(*ss))

            def qcopy(n):
                Qc_scr[pl.ds(zb + n * HD, HD), :] = pltpu.bitcast(q_next[:, n*W:(n+1)*W], U32)

            def qk(n, ci):
                t = st[n]
                nxt = n >= nt
                assert prologue or n < NB or (n - NB) // N in done['p'], ('S hazard', n)
                if nxt: assert prologue or done['k'] == kpieces
                if nxt:
                    if 'q' not in t: t['q'] = q_next[:, (n-nt)*W:(n-nt+1)*W]
                    q = t['q']
                else:
                    q = pltpu.bitcast(Qc_scr[pl.ds(zb + n * HD, HD), :], BF16)
                w12 = q[0:128]; w23 = q[64:192]
                w13 = jnp.concatenate([q[0:64], q[128:192]], axis=0)
                r0 = offs[ci]; R = sizes[ci]
                Lr = Ln_scr if nxt else Lc_scr
                ld = lambda i: pltpu.bitcast(Lr[pl.ds(zb + i * LSZ + r0 // 2, R // 2), :], BF16)
                p3 = jnp.dot(ld(0), w12, preferred_element_type=F32)
                p1 = jnp.dot(ld(1), w23, preferred_element_type=F32)
                p2 = jnp.dot(ld(2), w13, preferred_element_type=F32)
                sa = p1 + p3; sb = p2 + p3
                Sr = S_refs[n % NB]
                Sr[r0:r0+R, :] = sa
                Sr[HS+r0:HS+r0+R, :] = sb
                sab = jnp.maximum(sa, sb).reshape(R // 8, 8, W)
                for gi in range(ngv[ci]):
                    gm = sab[gi*GV:(gi+1)*GV].max(axis=0)
                    Sr[S + 8 + (goff[ci] + gi) * 8:S + 16 + (goff[ci] + gi) * 8, :] = gm
                    t['m'] = jnp.maximum(t['m'], gm) if 'm' in t else gm
                if ci == nch - 1:
                    t['m'] = jnp.broadcast_to(jnp.max(t['m'], axis=0, keepdims=True), (8, W))
                    Sr[s_fence, :] = t['m']
                    done['q'].add(n)
                    if not nxt and not final: qcopy(n)
                return p3

            def ecl(idx, x):
                n, u = divmod(idx, NEC)
                assert n in done['q'], ("e before q", n)
                t = st[n]
                g0 = u * 8; g1 = min(NGV, g0 + 8)
                s = S_refs[n % NB][S + 8 + g0 * 8:S + 8 + g1 * 8, :].reshape(g1 - g0, 8, W)
                m, = gate(x, t['m'])
                e = jnp.exp2(s - m[None]).sum(axis=0)
                t['e'] = t['e'] + e if 'e' in t else e
                if u == NEC - 1:
                    l = jnp.sum(t['e'], axis=0, keepdims=True)
                    t['M'] = t['m'] + jnp.broadcast_to(jnp.log2(l), (8, W))
                    del t['m'], t['e']

            def pcl(idx, x):
                T, k = divmod(idx, NCL)
                slab, sub = divmod(k, nsub)
                Br = B_refs[T % NBB]
                assert prologue or T < NBB or (T - NBB) in done['m'], ('B hazard', T)
                r0 = slab * 16
                qs = sorted(set(q for _, i, j in subs[sub] for q in (i, j)))
                Ms = dict(zip(qs, gate(x, *[st[N*T + q]['M'] for q in qs])))
                def b(kb, q):
                    return [jnp.exp2(S_refs[(N*T + q) % NB][pl.ds(kb * KB + r0 + odd, 8, stride=2), :] - Ms[q]) for odd in range(2)]
                def put_b(p, ab):
                    off = pidx[p] * (KB // 2) + r0 // 2
                    Br[off:off + 8, :] = pack(*ab)
                addv = lambda a, v: [a[t] + v[t] for t in range(2)]
                subv = lambda a, v: [a[t] - v[t] for t in range(2)]
                def ladd(q, v):
                    t = st[N*T + q]
                    t['l'] = t['l'] + v if 'l' in t else v
                for kd, i, j in subs[sub]:
                    if kd == 'd':
                        for q in (i, j):
                            pst['e', q] = pst['f', q] = b(q, q); pst['n', q] = 1
                    else:
                        bij = b(i, j); bji = b(j, i)
                        upd = subv if sgn(i, j) > 0 else addv
                        put_b(('x', i, j), bij); put_b(('y', i, j), bji)
                        put_b(('s', i, j), subv(bij, bji))
                        pst['e', i] = upd(pst['e', i], bij); pst['e', j] = upd(pst['e', j], bji)
                        pst['f', i] = upd(pst['f', i], bji); pst['f', j] = upd(pst['f', j], bij)
                        pst['n', i] += 1; pst['n', j] += 1
                    for q in (i, j):
                        if pst['n', q] == N // 2:
                            ev = pst['f', q][0] + pst['f', q][1]
                            ladd(q, ev + ev)
                        if pst['n', q] == N:
                            fi = pst.pop(('f', q)); del pst['n', q]
                            put_b(('e', q, q), pst.pop(('e', q))); put_b(('f', q, q), fi)
                            t = st[N*T + q]
                            t['l'] = t['l'] - (fi[0] + fi[1])
                if k == NCL - 1:
                    Br[b_fence, :] = pltpu.bitcast(st[N*T]['M'], U32)
                    for q in range(N):
                        t = st[N*T + q]
                        del t['M']
                        t['l'] = jnp.broadcast_to(1.0 / jnp.sum(t['l'], axis=0, keepdims=True), (8, W))
                    done['p'].add(T)

            def mgroup(g):
                T, r = divmod(g, GPT); pi, j = divmod(r, ng)
                assert T in done['p'], ("m before p", T)
                a = pltpu.bitcast(Ac_scr[pl.ds(zb + (pi * ng + j) * (HD // 2), HD // 2), :], BF16)
                b = pltpu.bitcast(B_refs[T % NBB][pi*(KB//2) + j*64:pi*(KB//2) + (j+1)*64, :], BF16)
                oj = jnp.dot(a, b, preferred_element_type=F32)
                cs = cst[T]
                p = prods[pi]
                cs[p] = oj if j == 0 else cs[p] + oj
                if j == ng - 1 and p[0] in 'ef':
                    q = p[1]
                    q0 = (N*T + q) * W
                    others = [(i, -1.0, cs['x', i, q]) for i in range(q)] + [(jj, sgn(q, jj), cs['y', q, jj]) for jj in range(q + 1, N)]
                    add = lambda acc, sg, v: acc + v if sg > 0 else acc - v
                    if p[0] == 'e':
                        g_ = cs[p]
                        for jj in reversed(range(q + 1, N)):
                            sg = sgn(q, jj)
                            g_ = add(add(g_, -sg, cs['x', q, jj]), sg, cs['s', q, jj])
                        for i in reversed(range(q)):
                            g_ = g_ + cs['y', i, q] + cs['s', i, q]
                        cs['g', q] = g_
                        c1 = g_
                        for _, sg, v in others: c1 = add(c1, sg, v)
                        oT_ref[0:HD, q0:q0+W] = (c1 * st[N*T + q]['l'][0:1]).astype(oT_ref.dtype)
                    else:
                        c2 = cs[p] - lam[q] * cs['g', q]
                        for t_, sg, v in others: c2 = c2 - (sg * lam[t_]) * v
                        oT_ref[HD:D, q0:q0+W] = (c2 * st[N*T + q]['l'][0:1]).astype(oT_ref.dtype)
                        if q == N - 1: done['m'].add(T)
                return oj

            def live_keys(n):
                T = n // N
                ks = []
                qdone = max(0, min(nch, LQ_ - n * nch))
                edone = max(0, min(NEC, LE_ - n * NEC))
                pdone = max(0, min(NCL, LP_ - T * NCL))
                if qdone > 0 and edone < NEC: ks.append('m')
                if 0 < edone < NEC: ks.append('e')
                if edone == NEC and pdone < NCL: ks.append('M')
                if pdone > 0: ks.append('l')
                return ks

            if prologue:
                kprep(0, HS)
                for i in range(NV): vprep(i, None)
                for n in range(LQ_ // nch, nt): qcopy(n)
            else:
                Lc_scr[pl.ds(zb, 3 * LSZ), :] = Ln_scr[pl.ds(zb, 3 * LSZ), :]
                Ac_scr[pl.ds(zb, ASZ), :] = An_scr[pl.ds(zb, ASZ), :]
                for n in range(NSTATE):
                    for key in live_keys(n):
                        st[n][key] = st_scr[n * 4 + KEYS.index(key)]
                    if LQ_ >= (n + 1) * nch: done['q'].add(n)
                    if LP_ >= (n // N + 1) * NCL: done['p'].add(n // N)
            pw = HS // kpieces
            last_r = None
            for pos, (kd, idx, s0, sz) in enumerate(order):
                if kd == 'q':
                    n, ci = divmod(idx + LQ_, nch)
                    if (not prologue or n >= nt) and (not final or n < nt):
                        res[pos] = qk(n, ci); last_r = pos
                elif not prologue:
                    res[pos] = mgroup(idx); last_r = pos
                for tk, ti, tpos, vr in after[pos]:
                    lim = NC if tk == 'p' else nt * NEC
                    if prologue and (tk in 'kv' or ti < lim): continue
                    if final and (tk in 'kv' or ti >= lim): continue
                    if tpos not in res:
                        tpos = last_r; vr = min(vr, res[tpos].shape[0] // 8 - 1)
                    x = res[tpos][8*vr:8*vr+8]
                    if tk == 'e': ecl(ti, x)
                    elif tk == 'p': pcl(ti, x)
                    elif tk == 'v': vprep(ti, x)
                    else:
                        kprep(ti * pw, (ti + 1) * pw); done['k'] += 1
            assert not pst
            if not final:
                for n in range(NSTATE):
                    keys = [k for k in st[nt + n] if k != 'q']
                    assert sorted(keys) == sorted(live_keys(n)), (n, keys, live_keys(n))
                    for key in keys:
                        st_scr[n * 4 + KEYS.index(key)] = st[nt + n][key]

        @pl.when(h == 0)
        def _():
            z_ref[0] = 0
            body('first')
        NH = pl.num_programs(0) - 1
        if last:
            @pl.when(jnp.logical_and(h > 0, h < NH))
            def _():
                body('main')
            @pl.when(h == NH)
            def _():
                body('last')
        else:
            @pl.when(h > 0)
            def _():
                body('main')

    @jax.jit
    def f(q, k, v):
        B, H, S_, D = q.shape
        NH = B * H
        qT = jnp.swapaxes(q, 2, 3).reshape(NH, D, S)
        kT = jnp.swapaxes(k, 2, 3).reshape(NH, D, S)
        vT = jnp.swapaxes(v, 2, 3).reshape(NH, D, S)
        cur = lambda g: (jnp.maximum(g - 1, 0), 0, 0)
        nxt = lambda g: (jnp.minimum(g, NH - 1), 0, 0)
        oT = pl.pallas_call(
            kern,
            grid=(NH + 1,),
            in_specs=[pl.BlockSpec((None, D, S), nxt)] * 3,
            out_specs=pl.BlockSpec((None, D, S), cur),
            out_shape=jax.ShapeDtypeStruct((NH, D, S), q.dtype),
            scratch_shapes=[pltpu.SMEM((1,), jnp.int32),
                            pltpu.VMEM((3 * (S // 4), 128), U32), pltpu.VMEM((3 * (S // 4), 128), U32),
                            pltpu.VMEM((NP * ng * (D // 4), 128), U32), pltpu.VMEM((NP * ng * (D // 4), 128), U32),
                            pltpu.VMEM((nt * (D // 2), 128), U32),
                            pltpu.VMEM((8, 128), F32), pltpu.VMEM((NSTATE * 4, 8, 128), F32)]
                           + [pltpu.VMEM((S + 8 + 8 * NGV, W), F32) for _ in range(NB)]
                           + [pltpu.VMEM((NP * (KB // 2) + 8, 128), U32) for _ in range(NBB)],
            compiler_params=pltpu.CompilerParams(dimension_semantics=("arbitrary",),
                                                 vmem_limit_bytes=100*1024*1024),
        )(qT, kT, vT)
        return jnp.swapaxes(oT.reshape(B, H, D, S), 2, 3)
    return f


_impl = make(vt0=3000, psq=0.8)


@jax.jit
def pallas_standalone__mha_softmax__prompt_kernel(q: jax.Array, k: jax.Array, v: jax.Array):
    return _impl(q, k, v)
```

```python
import bisect
import math
import jax, jax.numpy as jnp
import jax.experimental.pallas as pl
import jax.experimental.pallas.tpu as pltpu

F32 = jnp.float32
BF16 = jnp.bfloat16
U32 = jnp.uint32


def make(N=4, CH=208, mQL=150, mLP=150, mPM=500, tail=250, NB=16, NBB=4, kpieces=8, kt0=600, kt1=6000,
         vt0=500, vt1=9000, mearly=0, GV=4, espan=500, mC=300, cspan=4500, psq=0.8, pv0=14, pvn=8, kdl=0, rscr=False, nobc=True, opos=0, ipos=(0, 0, 0), lpad=0, rrows=8, zal=8, pmode=2, QA=512, om=False, lsz=512, seqv=0, pordv=0, toff=0, foldc=False, csz=4, verbose=False):
    W = 128; G = 96
    S = 2048; HS = S // 2; nt = S // W; nT = nt // N
    KB = S // N; ng = KB // 128
    NSTATE = 12
    KEYS = ('m', 'e', 'M', 'l')
    lam = [1.0 / math.tan(math.pi * (i + 1) / (N + 1)) for i in range(N)]
    sgn = lambda i, j: 1.0 if (i + j) % 2 == 1 else -1.0
    pairs = [(i, j) for i in range(N) for j in range(i + 1, N)]
    prods = []
    for i in range(N):
        for j in range(i + 1, N):
            prods += [('s', i, j), ('x', i, j), ('y', i, j)]
        prods += [('e', i, i), ('f', i, i)]
    if pordv == 1:
        for k in range(len(prods) - 2):
            if prods[k][0] == 'e' and prods[k + 1][0] == 'f' and prods[k + 2][0] != 'f':
                prods[k + 1], prods[k + 2] = prods[k + 2], prods[k + 1]
    NP = len(prods); pidx = {p: k for k, p in enumerate(prods)}
    if N == 2:
        subs = [[('d', 0, 1), ('p', 0, 1)]] if csz == 8 else [[('d', 0, 1)], [('p', 0, 1)]]
    else:
        seq = [('d', 0, 2), ('p', 0, 2), ('d', 1, 3), ('p', 1, 3), ('p', 0, 1), ('p', 2, 3), ('p', 0, 3), ('p', 1, 2)]
        if seqv == 1: seq = [('d', 0, 2), ('d', 1, 3), ('p', 0, 2), ('p', 1, 3), ('p', 0, 1), ('p', 0, 3), ('p', 2, 3), ('p', 1, 2)]
        if seqv == 2: seq = [('d', 0, 2), ('p', 0, 2), ('d', 1, 3), ('p', 1, 3), ('p', 0, 1), ('p', 0, 3), ('p', 1, 2), ('p', 2, 3)]
        subs = [[x] for x in seq] if csz == 4 else [seq[0:2], seq[2:4], seq[4:6], seq[6:8]]
    nsub = len(subs)
    sizes = [CH] * (HS // CH) + ([HS % CH] if HS % CH else [])
    nch = len(sizes); offs = [sum(sizes[:i]) for i in range(nch)]
    NQ = nt * nch; GPT = NP * ng; NM = nT * GPT
    TOT = (3 * HS * nt + NM * G) // 4
    PER = TOT / nT
    NCL = (KB // 16) * nsub
    ngv = [-(-(sz // 8) // GV) for sz in sizes]
    goff = [sum(ngv[:i]) for i in range(nch)]; NGV = sum(ngv)
    NEC = -(-NGV // 8)
    lead_p = PER + mPM
    lead_q = lead_p + PER + mLP + espan + mQL
    span = TOT - tail
    LP_ = int(math.ceil(lead_p / PER * NCL / nsub)) * nsub
    LQ_ = int(math.ceil(lead_q / (PER / N) * nch)) + 1

    order = []
    load = [0, 0, 0, 0]
    mi = 0; rows_done = 0
    def put(n):
        u = min(range(4), key=lambda u: load[u]); s = load[u]; load[u] += n; return s
    for k in range(NQ):
        sz = sizes[(k + LQ_) % nch]
        s = max(put(sz) for _ in range(3))
        order.append(('q', k, s, sz))
        rows_done += sz
        while mi < NM and min(load) + G // 2 <= sorted(load)[1]:
            order.append(('m', mi, put(G), G)); mi += 1
        target = rows_done * NM / (nt * HS - mearly)
        while mi + 4 <= target + 2 and mi + 4 <= NM:
            for _ in range(4):
                order.append(('m', mi, put(G), G)); mi += 1
    while mi < NM:
        order.append(('m', mi, put(G), G)); mi += 1
    cands = sorted((s + 8 * i, pos, i) for pos, (kd, idx, s, sz) in enumerate(order) for i in range(sz // 8))
    ctimes = [c[0] for c in cands]
    def pick(t):
        i = min(bisect.bisect_left(ctimes, t + toff), len(cands) - 1)
        best = min(cands[i:i + 4], key=lambda c: c[1])
        return best[1], best[2]
    tasks = []
    NC = NCL * nT
    for i in range(NC):
        tasks.append((((i // nsub) * nsub + 0.5 + (i % nsub) * psq) * span / NC, 'p', i + LP_))
    LE_ = None
    for kd, idx, s0, sz in order:
        if kd == 'q' and (idx + LQ_) % nch == nch - 1:
            n = (idx + LQ_) // nch
            for u in range(NEC):
                t = s0 + sz + mQL + u * espan / NEC
                if t >= span: t -= span; n_ = n - nt
                else: n_ = n
                tasks.append((t, 'e', n_ * NEC + u))
    LE_ = min(ti for _, kd, ti in tasks if kd == 'e')
    NCC = N * 12
    for T in range(-1, nT - 1):
        for u in range(NCC):
            tasks.append(((T + 1) * PER + mC + u * cspan / NCC, 'c', (T + 1) * NCC + u))
    for i in range(kpieces):
        tasks.append((kt0 + i * (kt1 - kt0) / kpieces, 'k', i))
    nv = 6
    vsub = len(pairs) + 1
    NV = ng * nv * vsub
    for i in range(NV):
        tasks.append((vt0 + i * (vt1 - vt0) / NV, 'v', i))
    tasks.sort()
    after = [[] for _ in order]
    cur = 0
    for t, kd, idx in tasks:
        pos, vr = pick(t)
        cur = max(cur, pos)
        after[cur].append((kd, idx, pos, vr))
    if verbose:
        print("TOT", TOT, "LQ", LQ_, "LE", LE_, "NEC", NEC, "LP", LP_, "load", load, "nch", nch, "NP", NP)

    def kern(q_hbm, k_hbm, v_hbm, o_hbm, ibuf, obuf, z_ref, Lc_scr, Ln_scr, Ac_scr, An_scr, Qc_scr, st_scr,
             isem, osem, *rest):
        S_refs = rest[:NB]; B_refs = rest[NB:NB + NBB]; R_refs = rest[NB + NBB:]
        NH, D = q_hbm.shape[0], q_hbm.shape[1]
        HD = D // 2
        c = (D ** -0.5) * math.log2(math.e)
        h = pl.program_id(0)
        BROWS = -(-NP // 2) * (KB // 2)
        ASZ = NP * (ng // 2) * (HD // 2)

        def body(mode):
            prologue = mode == 'first'
            final = mode == 'last'
            z = z_ref[0]
            zb = pl.multiple_of(z * zal, zal)
            slot = 0 if prologue else h % 2
            q_next, k_next, v_next = ibuf.at[slot, 0], ibuf.at[slot, 1], ibuf.at[slot, 2]
            oT_ref = obuf.at[1 - slot]
            def in_copy(i, head, sl, sem):
                return pltpu.make_async_copy((q_hbm, k_hbm, v_hbm)[i].at[head], ibuf.at[sl, i], isem.at[sem])
            def out_copy(head, sl, T=None):
                if T is None:
                    return pltpu.make_async_copy(obuf.at[sl], o_hbm.at[head], osem.at[0])
                cols = pl.ds(T * N * W, N * W)
                return pltpu.make_async_copy(obuf.at[sl, :, cols], o_hbm.at[head, :, cols], osem.at[1 + T])
            LSZ = lsz
            s_fence = pl.ds(pl.multiple_of(S + z * 8, 8), 8)
            r_fence = pl.ds(pl.multiple_of(NP * HD + z * 8, 8), 8)
            b_fence = pl.ds(pl.multiple_of(BROWS + z * 8, 8), 8)
            st = [dict() for _ in range(nt + NSTATE)]
            cst = [dict() for _ in range(nT)]
            pst = {}
            res = {}
            deadl = []
            curpos = [0]
            done = dict(k=0, q=set(), p=set(), m=set(), c=set())

            def gate(x, *ms):
                if x is None: return list(ms)
                cnd = x > jnp.inf
                return [jnp.where(cnd, x if m.dtype == F32 else pltpu.bitcast(x, m.dtype), m) for m in ms]

            def kprep(c0, c1):
                a1, a2, a3 = [k_next[r:r + 64, c0:c1] for r in (0, 64, 128)]
                b1, b2, b3 = [k_next[r:r + 64, HS + c0:HS + c1] for r in (0, 64, 128)]
                d1 = a2.astype(F32) - b2.astype(F32)
                d2 = b1.astype(F32) - a1.astype(F32)
                if foldc:
                    cat = lambda x, y: (jnp.concatenate([x.astype(F32), y.astype(F32)], axis=0) * c).astype(BF16)
                else:
                    cat = lambda x, y: jnp.concatenate([x.astype(BF16), y.astype(BF16)], axis=0)
                rr = lambda i: pl.ds(zb + i * LSZ + c0 // 2, (c1 - c0) // 2)
                Ln_scr[rr(0), :] = pltpu.bitcast(cat(a1, b2).T, U32)
                Ln_scr[rr(1), :] = pltpu.bitcast(cat(d1, a3).T, U32)
                Ln_scr[rr(2), :] = pltpu.bitcast(cat(d2, b3).T, U32)

            An16 = An_scr.bitcast(BF16)
            def gate16(x, v):
                if x is None: return v
                x2 = jnp.concatenate([x, x], axis=0)
                return jnp.where(x2 > jnp.inf, x2, v)

            def vprep(idx, x):
                pos_, sub = divmod(idx, vsub)
                j, r = divmod(pos_, nv)
                def ldv(half, kblk):
                    r0 = half * HD + 16 * r; c0 = kblk * KB + j * 128
                    return v_next[r0:r0 + 16, c0:c0 + 128]
                ldf = lambda half, kblk: ldv(half, kblk).astype(F32)
                def put_a(p, u):
                    ao = ((pidx[p] * ng + j) // 2) * HD + 16 * r
                    An16[ao:ao + 16, (j % 2) * W:(j % 2 + 1) * W] = u.astype(BF16)
                if sub == len(pairs):
                    for i in range(N):
                        a1 = gate16(x, ldf(0, i))
                        put_a(('e', i, i), a1)
                        put_a(('f', i, i), lam[i] * a1 + ldf(1, i))
                else:
                    i, jj = pairs[sub]
                    tau = sgn(i, jj); d = lam[i] - lam[jj]
                    a1i, a2i, a1j, a2j = gate16(x, ldf(0, i)), gate16(x, ldf(1, i)), ldf(0, jj), ldf(1, jj)
                    u = a1i + a1j if tau > 0 else a1i - a1j
                    w = a2i + a2j if tau > 0 else a2i - a2j
                    xn = u * (lam[jj] / d) + w * (1.0 / d)
                    put_a(('x', i, jj), xn); put_a(('y', i, jj), u + xn); put_a(('s', i, jj), a1i + xn)

            def qcopy(n):
                Qc_scr[pl.ds(zb + n * HD, HD), :] = pltpu.bitcast(q_next[:, n*W:(n+1)*W], U32)

            def qk(n, ci):
                t = st[n]
                nxt = n >= nt
                assert prologue or n < NB or (n - NB) // N in done['p'], ('S hazard', n)
                if nxt: assert prologue or done['k'] == kpieces
                if nxt:
                    if 'q' not in t: t['q'] = q_next[:, (n-nt)*W:(n-nt+1)*W]
                    q = t['q']
                else:
                    q = pltpu.bitcast(Qc_scr[pl.ds(zb + n * HD, HD), :], BF16)
                w12 = q[0:128]; w23 = q[64:192]
                w13 = jnp.concatenate([q[0:64], q[128:192]], axis=0)
                r0 = offs[ci]; R = sizes[ci]
                Lr = Ln_scr if nxt else Lc_scr
                ld = lambda i: pltpu.bitcast(Lr[pl.ds(zb + i * LSZ + r0 // 2, R // 2), :], BF16)
                p3 = jnp.dot(ld(0), w12, preferred_element_type=F32)
                p1 = jnp.dot(ld(1), w23, preferred_element_type=F32)
                p2 = jnp.dot(ld(2), w13, preferred_element_type=F32)
                sa = p1 + p3; sb = p2 + p3
                if not foldc:
                    sa = sa * c; sb = sb * c
                Sr = S_refs[n % NB]
                Sr[r0:r0+R, :] = sa
                Sr[HS+r0:HS+r0+R, :] = sb
                sab = jnp.maximum(sa, sb).reshape(R // 8, 8, W)
                for gi in range(ngv[ci]):
                    gm = sab[gi*GV:(gi+1)*GV].max(axis=0)
                    Sr[S + 8 + (goff[ci] + gi) * 8:S + 16 + (goff[ci] + gi) * 8, :] = gm
                    t['m'] = jnp.maximum(t['m'], gm) if 'm' in t else gm
                if ci == nch - 1:
                    t['m'] = jnp.broadcast_to(jnp.max(t['m'], axis=0, keepdims=True), (8, W))
                    Sr[s_fence, :] = t['m']
                    done['q'].add(n)
                    if not nxt and not final: qcopy(n)
                return p3

            def ecl(idx, x):
                n, u = divmod(idx, NEC)
                assert n in done['q'], ("e before q", n)
                t = st[n]
                g0 = u * 8; g1 = min(NGV, g0 + 8)
                s = S_refs[n % NB][S + 8 + g0 * 8:S + 8 + g1 * 8, :].reshape(g1 - g0, 8, W)
                m, = gate(x, t['m'])
                e = jnp.exp2(s - m[None]).sum(axis=0)
                t['e'] = t['e'] + e if 'e' in t else e
                if u == NEC - 1:
                    l = jnp.sum(t['e'], axis=0, keepdims=True)
                    t['M'] = t['m'] + jnp.broadcast_to(jnp.log2(l), (8, W))
                    del t['m'], t['e']

            def pcl(idx, x):
                T, k = divmod(idx, NCL)
                slab, sub = divmod(k, nsub)
                Br = B_refs[T % NBB]
                assert prologue or T < NBB or (T - NBB) in done['m'], ('B hazard', T)
                r0 = slab * 16
                qs = sorted(set(q for _, i, j in subs[sub] for q in (i, j)))
                Ms = dict(zip(qs, gate(x, *[st[N*T + q]['M'] for q in qs])))
                def b(kb, q):
                    s = S_refs[(N*T + q) % NB][kb * KB + r0:kb * KB + r0 + 16, :].reshape(2, 8, W)
                    return jnp.exp2(s - Ms[q][None])
                B16 = Br.bitcast(BF16)
                def put_b(p, v):
                    off = (pidx[p] // 2) * KB + r0; cb = (pidx[p] % 2) * W
                    B16[off:off + 16, cb:cb + W] = v.reshape(16, W).astype(BF16)
                addv = lambda a, v: a + v
                subv = lambda a, v: a - v
                def ladd(q, v):
                    t = st[N*T + q]
                    t['l'] = t['l'] + v if 'l' in t else v
                for kd, i, j in subs[sub]:
                    if kd == 'd':
                        for q in (i, j):
                            pst['e', q] = pst['f', q] = b(q, q); pst['n', q] = 1
                    else:
                        bij = b(i, j); bji = b(j, i)
                        upd = subv if sgn(i, j) > 0 else addv
                        put_b(('x', i, j), bij); put_b(('y', i, j), bji)
                        put_b(('s', i, j), subv(bij, bji))
                        pst['e', i] = upd(pst['e', i], bij); pst['e', j] = upd(pst['e', j], bji)
                        pst['f', i] = upd(pst['f', i], bji); pst['f', j] = upd(pst['f', j], bij)
                        pst['n', i] += 1; pst['n', j] += 1
                    for q in (i, j):
                        if pst['n', q] == N // 2:
                            ev = pst['f', q][0] + pst['f', q][1]
                            ladd(q, ev + ev)
                        if pst['n', q] == N:
                            fi = pst.pop(('f', q)); del pst['n', q]
                            put_b(('e', q, q), pst.pop(('e', q))); put_b(('f', q, q), fi)
                            t = st[N*T + q]
                            t['l'] = t['l'] - (fi[0] + fi[1])
                if k == NCL - 1:
                    Br[b_fence, 0:W] = pltpu.bitcast(st[N*T]['M'], U32)
                    for q in range(N):
                        t = st[N*T + q]
                        del t['M']
                        t['l'] = jnp.broadcast_to(1.0 / jnp.sum(t['l'], axis=0, keepdims=True), (8, W))
                    done['p'].add(T)

            def mgroup(g):
                T, r = divmod(g, GPT); pi, j = divmod(r, ng)
                assert T in done['p'], ("m before p", T)
                a = Ac_scr[pl.ds(zb + (j % 2) * ASZ + ((pi * ng + j) // 2) * (HD // 2), HD // 2), :]
                if deadl and deadl[0][0] <= curpos[0]:
                    a = jnp.concatenate([a[0:8] | deadl.pop(0)[1], a[8:]], axis=0)
                a = pltpu.bitcast(a, BF16)
                bo = (pi // 2) * (KB // 2) + j * 64
                b = pltpu.bitcast(B_refs[T % NBB][bo:bo + 64, (pi % 2) * W:(pi % 2 + 1) * W], BF16)
                oj = jnp.dot(a, b, preferred_element_type=F32)
                cs = cst[T]
                p = prods[pi]
                cs[p] = oj if j == 0 else cs[p] + oj
                if j == 0: assert T < 1 or (T - 2) in done['c'], ('R hazard', T)
                if j == ng - 1:
                    R_refs[T % 2][pi * HD:(pi + 1) * HD, :] = cs.pop(p)
                    if pi == NP - 1:
                        done['m'].add(T)
                        if not (final and T == nT - 1): R_refs[T % 2][r_fence, :] = oj[0:8]
                    if final and T == nT - 1 and p[0] == 'f':
                        for r in range(12): ccl(nT * NCC + p[1] * 12 + r, oj[8*r:8*r+8])
                return oj

            def ccl(idx, x):
                T, u = divmod(idx, NCC); T -= 1
                q, r = divmod(u, 12)
                assert T < 0 or T in done['m'] or (final and T == nT - 1), ('c before m', T)
                Rr = R_refs[T % 2]
                R = lambda *p: Rr[pidx[p] * HD + 8 * r:pidx[p] * HD + 8 * r + 8, :]
                add = lambda acc, sg, v: acc + v if sg > 0 else acc - v
                others = [(i, -1.0, R('x', i, q)) for i in range(q)] + [(jj, sgn(q, jj), R('y', q, jj)) for jj in range(q + 1, N)]
                g_, = gate(x, R('e', q, q))
                for jj in range(q + 1, N):
                    g_ = add(add(g_, sgn(q, jj), R('s', q, jj)), -sgn(q, jj), R('x', q, jj))
                for i in range(q):
                    g_ = (g_ + R('y', i, q)) + R('s', i, q)
                c1 = g_
                c2 = R('f', q, q) - lam[q] * g_
                for t_, sg, v in others:
                    c1 = add(c1, sg, v)
                    c2 = c2 - (sg * lam[t_]) * v
                if T < 0:
                    li = st_scr[NSTATE * 4 + q]; ob = obuf.at[slot]
                else:
                    li = st[N*T + q]['l']; ob = oT_ref
                q0 = (N * (T % nT) + q) * W
                ob[8*r:8*r+8, q0:q0+W] = (c1 * li).astype(ob.dtype)
                ob[HD+8*r:HD+8*r+8, q0:q0+W] = (c2 * li).astype(ob.dtype)
                if u == NCC - 1:
                    done['c'].add(T)
                    if T < 0:
                        @pl.when(h > 1)
                        def _():
                            out_copy(h - 2, slot).start()
                    elif final:
                        out_copy(h - 1, 1 - slot, T).start()

            def live_keys(n):
                T = n // N
                ks = []
                qdone = max(0, min(nch, LQ_ - n * nch))
                edone = max(0, min(NEC, LE_ - n * NEC))
                pdone = max(0, min(NCL, LP_ - T * NCL))
                if qdone > 0 and edone < NEC: ks.append('m')
                if 0 < edone < NEC: ks.append('e')
                if edone == NEC and pdone < NCL: ks.append('M')
                if pdone > 0: ks.append('l')
                return ks

            h1 = jnp.minimum(h + 1, NH - 1)
            if prologue:
                if kdl: Ln_scr[3 * LSZ:3 * LSZ + 8, :] = jnp.zeros((8, 128), U32)
                if pmode == 0:
                    for i in (1, 0, 2): in_copy(i, 0, 0, 1 + i).start()
                    for i in range(3): in_copy(i, h1, 1, 0).start()
                    in_copy(1, 0, 0, 2).wait()
                    kprep(0, HS)
                    in_copy(0, 0, 0, 1).wait()
                elif pmode == 1:
                    in_copy(1, 0, 0, 2).start()
                    in_copy(0, 0, 0, 1).start()
                    in_copy(1, 0, 0, 2).wait()
                    in_copy(2, 0, 0, 3).start()
                    kprep(0, HS)
                    in_copy(0, 0, 0, 1).wait()
                    for i in range(3): in_copy(i, h1, 1, 0).start()
                else:
                    qa = pltpu.make_async_copy(q_hbm.at[0, :, 0:QA], ibuf.at[0, 0, :, 0:QA], isem.at[1])
                    qb = pltpu.make_async_copy(q_hbm.at[0, :, QA:S], ibuf.at[0, 0, :, QA:S], isem.at[4])
                    in_copy(1, 0, 0, 2).start(); qa.start()
                    R_refs[(nT - 1) % 2][0:NP * HD, :] = jnp.zeros((NP * HD, W), F32)
                    for q in range(N): st_scr[NSTATE * 4 + q] = jnp.zeros((8, W), F32)
                    in_copy(1, 0, 0, 2).wait(); qa.wait()
                    qb.start(); in_copy(2, 0, 0, 3).start()
                    kprep(0, HS)
            else:
                for i in range(3): Lc_scr[pl.ds(zb + i * LSZ, HS // 2), :] = Ln_scr[pl.ds(zb + i * LSZ, HS // 2), :]
                for i in range(2): Ac_scr[pl.ds(zb + i * ASZ, ASZ), :] = An_scr[:, i * W:(i + 1) * W]
                for n in range(NSTATE):
                    for key in live_keys(n):
                        st[n][key] = st_scr[n * 4 + KEYS.index(key)]
                    if LQ_ >= (n + 1) * nch: done['q'].add(n)
                    if LP_ >= (n // N + 1) * NCL: done['p'].add(n // N)
            pw = HS // kpieces
            last_r = None
            nq = 0; vdone = 0
            for pos, (kd, idx, s0, sz) in enumerate(order):
                curpos[0] = pos
                if not prologue:
                    for i in range(3):
                        if pos == ipos[i] and not final: in_copy(i, h1, 1 - slot, 0).start()
                if kd == 'q':
                    n, ci = divmod(idx + LQ_, nch)
                    if (not prologue or n >= nt) and (not final or n < nt):
                        res[pos] = qk(n, ci); last_r = pos
                        if prologue:
                            nq += 1
                            if nq == pv0:
                                in_copy(2, 0, 0, 3).wait()
                                if pmode == 2:
                                    assert nq <= (QA // W) * nch
                                    qb.wait()
                                    for i in range(3): in_copy(i, h1, 1, 0).start()
                            if nq == pv0 + 1:
                                for n2 in range(LQ_ // nch, nt): qcopy(n2)
                            if nq >= pv0:
                                nvr = res[pos].shape[0] // 8
                                for u in range(pvn):
                                    if vdone < NV:
                                        vr = (u * nvr) // pvn
                                        vprep(vdone, res[pos][8*vr:8*vr+8]); vdone += 1
                elif not prologue:
                    res[pos] = mgroup(idx); last_r = pos
                for tk, ti, tpos, vr in after[pos]:
                    lim = NC if tk == 'p' else nt * NEC
                    if prologue and (tk in 'kvc' or ti < lim): continue
                    if final and tk != 'c' and (tk in 'kv' or ti >= lim): continue
                    if tpos not in res:
                        tpos = last_r; vr = min(vr, res[tpos].shape[0] // 8 - 1)
                    x = res[tpos][8*vr:8*vr+8]
                    if tk == 'e': ecl(ti, x)
                    elif tk == 'p': pcl(ti, x)
                    elif tk == 'c': ccl(ti, x)
                    elif tk == 'v': vprep(ti, x)
                    else:
                        kprep(ti * pw, (ti + 1) * pw); done['k'] += 1
                        if kdl: deadl.append((pos + kdl, Ln_scr[pl.ds(pl.multiple_of(3 * LSZ + z_ref[1] * 8, 8), 8), :]))
            assert not pst and (not prologue or vdone == NV)
            if final:
                pass
            elif prologue:
                pass
            else:
                for q in range(N): st_scr[NSTATE * 4 + q] = st[nt - N + q]['l']
            if not final:
                for n in range(NSTATE):
                    keys = [k for k in st[nt + n] if k != 'q']
                    assert sorted(keys) == sorted(live_keys(n)), (n, keys, live_keys(n))
                    for key in keys:
                        st_scr[n * 4 + KEYS.index(key)] = st[nt + n][key]

            if not final:
                pltpu.make_async_copy(ibuf.at[1 - slot], ibuf.at[1 - slot], isem.at[0]).wait()
            if not prologue:
                @pl.when(h > 1)
                def _():
                    out_copy(h - 2, slot).wait()
            if final:
                for T in range(nT): out_copy(h - 1, 1 - slot, T).wait()

        @pl.when(h == 0)
        def _():
            z_ref[0] = 0
            z_ref[1] = 0
            if not om: body('first')
        @pl.when(jnp.logical_and(h > 0, h < NH))
        def _():
            body('main')
        @pl.when(h == NH)
        def _():
            if not om: body('last')
            else: z_ref[1] = 0

    @jax.jit
    def f(q, k, v):
        B, H, S_, D = q.shape
        NH = B * H
        qT = jnp.swapaxes(q, 2, 3).reshape(NH, D, S)
        kT = jnp.swapaxes(k, 2, 3).reshape(NH, D, S)
        vT = jnp.swapaxes(v, 2, 3).reshape(NH, D, S)
        oT = pl.pallas_call(
            kern,
            grid=(NH + 1,),
            in_specs=[pl.BlockSpec(memory_space=pl.ANY)] * 3,
            out_specs=pl.BlockSpec(memory_space=pl.ANY),
            out_shape=jax.ShapeDtypeStruct((NH, D, S), q.dtype),
            scratch_shapes=[pltpu.VMEM((2, 3, D, S), q.dtype), pltpu.VMEM((2, D, S), q.dtype), pltpu.SMEM((2,), jnp.int32),
                            pltpu.VMEM((-(-3 * lsz // 256) * 256, 128), U32), pltpu.VMEM((-(-3 * lsz // 256) * 256 + lpad, 128), U32),
                            pltpu.VMEM((NP * ng * (D // 4), 128), U32), pltpu.VMEM((NP * ng * (D // 8), 256), U32),
                            pltpu.VMEM((nt * (D // 2), 128), U32),
                            pltpu.VMEM((NSTATE * 4 + 16, 8, 128), F32)]
                           + [pltpu.SemaphoreType.DMA((5,)), pltpu.SemaphoreType.DMA((1 + nT,))]
                           + [pltpu.VMEM((S + 8 + 8 * NGV, W), F32) for _ in range(NB)]
                           + [pltpu.VMEM((-(-NP // 2) * (KB // 2) + 8, 256), U32) for _ in range(NBB)]
                           + [pltpu.VMEM((NP * (D // 2) + 8, 128), F32) for _ in range(2)],
            compiler_params=pltpu.CompilerParams(dimension_semantics=("arbitrary",),
                                                 vmem_limit_bytes=100*1024*1024, disable_bounds_checks=nobc),
        )(qT, kT, vT)
        return jnp.swapaxes(oT.reshape(B, H, D, S), 2, 3)
    return f


_impl = make(psq=1.0)


@jax.jit
def pallas_standalone__mha_softmax__prompt_kernel(q: jax.Array, k: jax.Array, v: jax.Array):
    return _impl(q, k, v)
```

```python
import bisect
import math

import jax
import jax.numpy as jnp
import jax.experimental.pallas as pl
import jax.experimental.pallas.tpu as pltpu

F32 = jnp.float32
BF16 = jnp.bfloat16
U32 = jnp.uint32

S = 2048
HD = 96
D = 2 * HD
W = 128
N = 4
HS = S // 2
NT = S // W
NS = NT // N
KB = S // N
NG = KB // 128
NB, NBB = 16, 4
NSTATE = 12
KEYS = ('m', 'e', 'M', 'l')

LAM = [1.0 / math.tan(math.pi * (i + 1) / (N + 1)) for i in range(N)]
PAIRS = [(i, j) for i in range(N) for j in range(i + 1, N)]
PRODS = []
for _i in range(N):
    for _j in range(_i + 1, N):
        PRODS += [('s', _i, _j), ('x', _i, _j), ('y', _i, _j)]
    PRODS += [('e', _i, _i), ('f', _i, _i)]
NP = len(PRODS)
PIDX = {p: k for k, p in enumerate(PRODS)}
SUBS = [('d', 0, 2), ('p', 0, 2), ('d', 1, 3), ('p', 1, 3), ('p', 0, 1), ('p', 0, 3), ('p', 1, 2), ('p', 2, 3)]
NSUB = len(SUBS)


def _sgn(i, j):
    return 1.0 if (i + j) % 2 == 1 else -1.0


CH = 208
GV = 4
SIZES = [CH] * (HS // CH) + [HS % CH]
NCH = len(SIZES)
OFFS = [sum(SIZES[:i]) for i in range(NCH)]
GPT = NP * NG
TOT = (3 * HS * NT + NS * GPT * HD) // 4
PER = TOT / NS
NCL = (KB // 16) * NSUB
NGVS = [-(-(sz // 8) // GV) for sz in SIZES]
GOFF = [sum(NGVS[:i]) for i in range(NCH)]
NGV = sum(NGVS)
NEC = -(-NGV // 8)
NCC = N * (HD // 8)
KPIECES = 8
VSUB = len(PAIRS) + 1
NV = NG * (HD // 16) * VSUB
QA = 512
PV0, PVN = 18, 10


def _plan(m_ql=200, m_lp=150, m_pm=600, tail=300, espan=450, m_c=250, cspan=5000,
          kt=(600, 6000), vt=(3000, 16000)):
    lead_p = PER + m_pm
    lead_q = lead_p + PER + m_lp + espan + m_ql
    span = TOT - tail
    lp = int(math.ceil(lead_p / PER * NCL / NSUB)) * NSUB
    lq = int(math.ceil(lead_q / (PER / N) * NCH)) + 1
    nm = NS * GPT
    order, load = [], [0, 0, 0, 0]

    def put(n):
        u = min(range(4), key=lambda u: load[u])
        load[u] += n
        return load[u] - n

    mi = rows = 0
    for k in range(NT * NCH):
        sz = SIZES[(k + lq) % NCH]
        order.append(('q', k, max(put(sz) for _ in range(3)), sz))
        rows += sz
        while mi < nm and min(load) + HD // 2 <= sorted(load)[1]:
            order.append(('m', mi, put(HD), HD)); mi += 1
        while mi + 4 <= rows * nm / (NT * HS) + 2 and mi + 4 <= nm:
            for _ in range(4):
                order.append(('m', mi, put(HD), HD)); mi += 1
    while mi < nm:
        order.append(('m', mi, put(HD), HD)); mi += 1

    tasks = [((i + 0.5) * span / (NCL * NS), 'p', i + lp) for i in range(NCL * NS)]
    for kd, idx, s0, sz in order:
        if kd == 'q' and (idx + lq) % NCH == NCH - 1:
            n = (idx + lq) // NCH
            for u in range(NEC):
                t = s0 + sz + m_ql + u * espan / NEC
                tasks.append((t - span, 'e', (n - NT) * NEC + u) if t >= span else (t, 'e', n * NEC + u))
    le = min(ti for _, kd, ti in tasks if kd == 'e')
    tasks += [(T * PER + m_c + u * cspan / NCC, 'c', T * NCC + u) for T in range(NS) for u in range(NCC)]
    tasks += [(kt[0] + i * (kt[1] - kt[0]) / KPIECES, 'k', i) for i in range(KPIECES)]
    tasks += [(vt[0] + i * (vt[1] - vt[0]) / NV, 'v', i) for i in range(NV)]
    tasks.sort()

    cands = sorted((s + 8 * i, pos, i) for pos, (_, _, s, sz) in enumerate(order) for i in range(sz // 8))
    times = [c[0] for c in cands]
    after, cur = [[] for _ in order], 0
    for t, kd, idx in tasks:
        i = min(bisect.bisect_left(times, t), len(cands) - 1)
        _, pos, vr = min(cands[i:i + 4], key=lambda c: c[1])
        cur = max(cur, pos)
        after[cur].append((kd, idx, pos, vr))
    return order, after, lq, le, lp


ORDER, AFTER, LQ, LE, LP = _plan()
BROWS = (NP // 2) * (KB // 2)
ASZ = NP * (NG // 2) * (HD // 2)
LSZ = HS // 2


def _live_keys(n):
    qdone = max(0, min(NCH, LQ - n * NCH))
    edone = max(0, min(NEC, LE - n * NEC))
    pdone = max(0, min(NCL, LP - (n // N) * NCL))
    ks = []
    if qdone > 0 and edone < NEC: ks.append('m')
    if 0 < edone < NEC: ks.append('e')
    if edone == NEC and pdone < NCL: ks.append('M')
    if pdone > 0: ks.append('l')
    return ks


def _gate(x, *ms):
    cnd = x > jnp.inf
    return [jnp.where(cnd, x, m) for m in ms]


def _kernel(q_hbm, k_hbm, v_hbm, o_hbm, ibuf, obuf, z_ref, Lc, Ln, Ac, An, Qc, st_scr, isem, osem, *rest):
    S_refs, B_refs, R_refs = rest[:NB], rest[NB:NB + NBB], rest[NB + NBB:]
    NH = q_hbm.shape[0]
    scale = (D ** -0.5) * math.log2(math.e)
    g = pl.program_id(0)

    def in_copy(i, head, par, sem):
        return pltpu.make_async_copy((q_hbm, k_hbm, v_hbm)[i].at[head], ibuf.at[par, i], isem.at[sem])

    def prefetch(par):
        head = jnp.minimum(g + 1, NH - 1)
        for i in range(3):
            in_copy(i, head, par, 0).start()

    def wait_inputs(par):
        pltpu.make_async_copy(ibuf.at[par], ibuf.at[par], isem.at[0]).wait()

    def out_copy(step, piece=None):
        if piece is None:
            return pltpu.make_async_copy(obuf.at[step % 2], o_hbm.at[step - 1], osem.at[0])
        cols = pl.ds(piece * N * W, N * W) if piece < NS - 1 else pl.ds((piece + (NS - 1) * (N - 1)) * W, W)
        return pltpu.make_async_copy(obuf.at[step % 2, :, cols], o_hbm.at[step - 1, :, cols], osem.at[1 + piece])

    def body(first, last):
        z = z_ref[0]
        zb = pl.multiple_of(z * 8, 8)
        fence = lambda r: pl.ds(pl.multiple_of(r + z * 8, 8), 8)
        par = 0 if first else g % 2
        q_next, k_next, v_next = [ibuf.at[par, i] for i in range(3)]
        st = [dict() for _ in range(NT + NSTATE)]
        acc, pst, res = {}, {}, {}
        done = dict(k=0, q=set(), p=set(), m=set(), c=set())

        def kprep(c0, c1):
            a1, a2, a3 = [k_next[r:r + 64, c0:c1] for r in (0, 64, 128)]
            b1, b2, b3 = [k_next[r:r + 64, HS + c0:HS + c1] for r in (0, 64, 128)]
            d1 = (a2.astype(F32) - b2.astype(F32)).astype(BF16)
            d2 = (b1.astype(F32) - a1.astype(F32)).astype(BF16)
            for i, (x, y) in enumerate(((a1, b2), (d1, a3), (d2, b3))):
                Ln[pl.ds(zb + i * LSZ + c0 // 2, (c1 - c0) // 2), :] = pltpu.bitcast(
                    jnp.concatenate([x, y], axis=0).T, U32)

        def vprep(idx, x):
            pos, sb = divmod(idx, VSUB)
            j, r = divmod(pos, HD // 16)
            x2 = jnp.concatenate([x, x], axis=0)

            def ldf(half, kblk):
                r0, c0 = half * HD + 16 * r, kblk * KB + j * 128
                return v_next[r0:r0 + 16, c0:c0 + 128].astype(F32)

            def put_a(p, u):
                ao = ((PIDX[p] * NG + j) // 2) * (HD // 2) + 8 * r
                An[ao:ao + 8, (j % 2) * W:(j % 2 + 1) * W] = pltpu.bitcast(u.astype(BF16), U32)

            if sb == len(PAIRS):
                for i in range(N):
                    a1, = _gate(x2, ldf(0, i))
                    put_a(('e', i, i), a1)
                    put_a(('f', i, i), LAM[i] * a1 + ldf(1, i))
            else:
                i, jj = PAIRS[sb]
                d = LAM[i] - LAM[jj]
                a1i, a2i = _gate(x2, ldf(0, i), ldf(1, i))
                a1j, a2j = ldf(0, jj), ldf(1, jj)
                u = a1i + a1j if _sgn(i, jj) > 0 else a1i - a1j
                w = a2i + a2j if _sgn(i, jj) > 0 else a2i - a2j
                xn = u * (LAM[jj] / d) + w * (1.0 / d)
                put_a(('x', i, jj), xn)
                put_a(('y', i, jj), u + xn)
                put_a(('s', i, jj), a1i + xn)

        def qcopy(n):
            Qc[pl.ds(zb + n * HD, HD), :] = pltpu.bitcast(q_next[:, n * W:(n + 1) * W], U32)

        def qk(n, ci):
            t, nxt = st[n], n >= NT
            assert first or n < NB or (n - NB) // N in done['p']
            if nxt:
                assert first or done['k'] == KPIECES
                if 'q' not in t:
                    t['q'] = q_next[:, (n - NT) * W:(n - NT + 1) * W]
                q = t['q']
            else:
                q = pltpu.bitcast(Qc[pl.ds(zb + n * HD, HD), :], BF16)
            r0, rows = OFFS[ci], SIZES[ci]
            lhs = lambda i: pltpu.bitcast((Ln if nxt else Lc)[pl.ds(zb + i * LSZ + r0 // 2, rows // 2), :], BF16)
            p3 = jnp.dot(lhs(0), q[0:128], preferred_element_type=F32)
            p1 = jnp.dot(lhs(1), q[64:192], preferred_element_type=F32)
            p2 = jnp.dot(lhs(2), jnp.concatenate([q[0:64], q[128:192]], axis=0), preferred_element_type=F32)
            sa = (p1 + p3) * scale
            sb = (p2 + p3) * scale
            Sr = S_refs[n % NB]
            Sr[r0:r0 + rows, :] = sa
            Sr[HS + r0:HS + r0 + rows, :] = sb
            sab = jnp.maximum(sa, sb).reshape(rows // 8, 8, W)
            for gi in range(NGVS[ci]):
                gm = sab[gi * GV:(gi + 1) * GV].max(axis=0)
                go = S + 8 + (GOFF[ci] + gi) * 8
                Sr[go:go + 8, :] = gm
                t['m'] = jnp.maximum(t['m'], gm) if 'm' in t else gm
            if ci == NCH - 1:
                t['m'] = jnp.broadcast_to(jnp.max(t['m'], axis=0, keepdims=True), (8, W))
                Sr[fence(S), :] = t['m']
                done['q'].add(n)
                if not nxt and not last:
                    qcopy(n)
            return p3

        def ecl(idx, x):
            n, u = divmod(idx, NEC)
            assert n in done['q']
            t = st[n]
            g0, g1 = u * 8, min(NGV, u * 8 + 8)
            s = S_refs[n % NB][S + 8 + g0 * 8:S + 8 + g1 * 8, :].reshape(g1 - g0, 8, W)
            m, = _gate(x, t['m'])
            e = jnp.exp2(s - m[None]).sum(axis=0)
            t['e'] = t['e'] + e if 'e' in t else e
            if u == NEC - 1:
                tot = jnp.sum(t.pop('e'), axis=0, keepdims=True)
                t['M'] = t.pop('m') + jnp.broadcast_to(jnp.log2(tot), (8, W))

        def pcl(idx, x):
            T, k = divmod(idx, NCL)
            slab, sb = divmod(k, NSUB)
            Br = B_refs[T % NBB]
            assert first or T < NBB or (T - NBB) in done['m']
            r0 = slab * 16
            kd, i, j = SUBS[sb]
            Ms = dict(zip((i, j), _gate(x, st[N * T + i]['M'], st[N * T + j]['M'])))

            def b(kb, q):
                s = S_refs[(N * T + q) % NB][kb * KB + r0:kb * KB + r0 + 16, :].reshape(2, 8, W)
                return jnp.exp2(s - Ms[q][None])

            def put_b(p, v):
                off, cb = (PIDX[p] // 2) * (KB // 2) + r0 // 2, (PIDX[p] % 2) * W
                Br[off:off + 8, cb:cb + W] = pltpu.bitcast(v.reshape(16, W).astype(BF16), U32)

            if kd == 'd':
                for q in (i, j):
                    pst['e', q] = pst['f', q] = b(q, q)
                    pst['n', q] = 1
            else:
                bij, bji = b(i, j), b(j, i)
                upd = (lambda a, v: a - v) if _sgn(i, j) > 0 else (lambda a, v: a + v)
                put_b(('x', i, j), bij)
                put_b(('y', i, j), bji)
                put_b(('s', i, j), bij - bji)
                pst['e', i], pst['e', j] = upd(pst['e', i], bij), upd(pst['e', j], bji)
                pst['f', i], pst['f', j] = upd(pst['f', i], bji), upd(pst['f', j], bij)
                pst['n', i] += 1
                pst['n', j] += 1
            for q in (i, j):
                t = st[N * T + q]
                if pst['n', q] == N // 2:
                    ev = pst['f', q][0] + pst['f', q][1]
                    t['l'] = t['l'] + (ev + ev) if 'l' in t else ev + ev
                if pst['n', q] == N:
                    fi = pst.pop(('f', q))
                    del pst['n', q]
                    put_b(('e', q, q), pst.pop(('e', q)))
                    put_b(('f', q, q), fi)
                    t['l'] = t['l'] - (fi[0] + fi[1])
            if k == NCL - 1:
                Br[fence(BROWS), 0:W] = pltpu.bitcast(st[N * T]['M'], U32)
                for q in range(N):
                    t = st[N * T + q]
                    del t['M']
                    t['l'] = jnp.broadcast_to(1.0 / jnp.sum(t['l'], axis=0, keepdims=True), (8, W))
                done['p'].add(T)

        def mgroup(gi):
            T, r = divmod(gi, GPT)
            pi, j = divmod(r, NG)
            assert T in done['p'] and (j > 0 or T < 1 or (T - 2) in done['c'])
            a = Ac[pl.ds(zb + (j % 2) * ASZ + ((pi * NG + j) // 2) * (HD // 2), HD // 2), :]
            bo = (pi // 2) * (KB // 2) + j * 64
            b = B_refs[T % NBB][bo:bo + 64, (pi % 2) * W:(pi % 2 + 1) * W]
            oj = jnp.dot(pltpu.bitcast(a, BF16), pltpu.bitcast(b, BF16), preferred_element_type=F32)
            acc['o'] = oj if j == 0 else acc['o'] + oj
            if j == NG - 1:
                R_refs[T % 2][pi * HD:(pi + 1) * HD, :] = acc.pop('o')
                inline = last and T == NS - 1
                if pi == NP - 1:
                    done['m'].add(T)
                    if not inline:
                        R_refs[T % 2][fence(NP * HD), :] = oj[0:8]
                if inline and PRODS[pi][0] == 'f':
                    for r in range(HD // 8):
                        ccl(NS * NCC + PRODS[pi][1] * (HD // 8) + r, oj[8 * r:8 * r + 8])
            return oj

        def ccl(idx, x):
            T, u = divmod(idx, NCC)
            T -= 1
            q, r = divmod(u, HD // 8)
            assert T < 0 or T in done['m'] or (last and T == NS - 1)
            Rr = R_refs[T % 2]
            R = lambda *p: Rr[PIDX[p] * HD + 8 * r:PIDX[p] * HD + 8 * r + 8, :]
            add = lambda a, sg, v: a + v if sg > 0 else a - v
            others = ([(i, -1.0, R('x', i, q)) for i in range(q)]
                      + [(jj, _sgn(q, jj), R('y', q, jj)) for jj in range(q + 1, N)])
            gq, = _gate(x, R('e', q, q))
            for jj in range(q + 1, N):
                gq = add(add(gq, _sgn(q, jj), R('s', q, jj)), -_sgn(q, jj), R('x', q, jj))
            for i in range(q):
                gq = (gq + R('y', i, q)) + R('s', i, q)
            c1 = gq
            c2 = R('f', q, q) - LAM[q] * gq
            for t_, sg, v in others:
                c1 = add(c1, sg, v)
                c2 = c2 - (sg * LAM[t_]) * v
            if T < 0:
                linv, ob = st_scr[NSTATE * 4 + q], obuf.at[(g - 1) % 2]
            else:
                linv, ob = st[N * T + q]['l'], obuf.at[g % 2]
            q0 = (N * (T % NS) + q) * W
            ob[8 * r:8 * r + 8, q0:q0 + W] = (c1 * linv).astype(ob.dtype)
            ob[HD + 8 * r:HD + 8 * r + 8, q0:q0 + W] = (c2 * linv).astype(ob.dtype)
            if u == NCC - 1:
                done['c'].add(T)
                if T < 0:
                    @pl.when(g > 1)
                    def _():
                        out_copy(g - 1).start()
                elif last and T < NS - 1:
                    out_copy(g, T).start()
            if last and T == NS - 1 and r == HD // 8 - 1:
                out_copy(g, T + q).start()

        if first:
            qa = pltpu.make_async_copy(q_hbm.at[0, :, 0:QA], ibuf.at[0, 0, :, 0:QA], isem.at[1])
            qb = pltpu.make_async_copy(q_hbm.at[0, :, QA:S], ibuf.at[0, 0, :, QA:S], isem.at[4])
            in_copy(1, 0, 0, 2).start()
            qa.start()
            in_copy(2, 0, 0, 3).start()
            qb.start()
            R_refs[(NS - 1) % 2][0:NP * HD, :] = jnp.zeros((NP * HD, W), F32)
            for q in range(N):
                st_scr[NSTATE * 4 + q] = jnp.zeros((8, W), F32)
            in_copy(1, 0, 0, 2).wait()
            qa.wait()
            kprep(0, HS)
        else:
            Lc[pl.ds(zb, 3 * LSZ), :] = Ln[pl.ds(zb, 3 * LSZ), :]
            for i in range(2):
                Ac[pl.ds(zb + i * ASZ, ASZ), :] = An[0:ASZ, i * W:(i + 1) * W]
            for n in range(NSTATE):
                for key in _live_keys(n):
                    st[n][key] = st_scr[n * 4 + KEYS.index(key)]
                if LQ >= (n + 1) * NCH: done['q'].add(n)
                if LP >= (n // N + 1) * NCL: done['p'].add(n // N)

        pw = HS // KPIECES
        last_r, nq, vdone = None, 0, 0
        for pos, (kd, idx, _, _) in enumerate(ORDER):
            if kd == 'q':
                n, ci = divmod(idx + LQ, NCH)
                if (not first or n >= NT) and (not last or n < NT):
                    res[pos] = qk(n, ci)
                    last_r = pos
                    if first:
                        nq += 1
                        if nq == PV0:
                            assert nq <= (QA // W) * NCH
                            in_copy(2, 0, 0, 3).wait()
                            qb.wait()
                            prefetch(1)
                        if nq == PV0 + 1:
                            for n2 in range(LQ // NCH, NT):
                                qcopy(n2)
                        for u in range(PVN if nq >= PV0 else 0):
                            if vdone < NV:
                                vr = (u * (res[pos].shape[0] // 8)) // PVN
                                vprep(vdone, res[pos][8 * vr:8 * vr + 8])
                                vdone += 1
            elif not first:
                res[pos] = mgroup(idx)
                last_r = pos
            for tk, ti, tpos, vr in AFTER[pos]:
                lim = NCL * NS if tk == 'p' else NT * NEC
                if first and (tk in 'kvc' or ti < lim): continue
                if last and tk != 'c' and (tk in 'kv' or ti >= lim): continue
                if tpos not in res:
                    tpos, vr = last_r, min(vr, res[last_r].shape[0] // 8 - 1)
                x = res[tpos][8 * vr:8 * vr + 8]
                if tk == 'k':
                    kprep(ti * pw, (ti + 1) * pw)
                    done['k'] += 1
                else:
                    dict(e=ecl, p=pcl, c=ccl, v=vprep)[tk](ti, x)
        assert not pst and (not first or vdone == NV)
        if not last:
            if not first:
                for q in range(N):
                    st_scr[NSTATE * 4 + q] = st[NT - N + q]['l']
            for n in range(NSTATE):
                assert sorted(k for k in st[NT + n] if k != 'q') == sorted(_live_keys(n))
                for key in _live_keys(n):
                    st_scr[n * 4 + KEYS.index(key)] = st[NT + n][key]

    def step(last):
        if not last:
            prefetch((g + 1) % 2)
        body(False, last)
        if not last:
            wait_inputs((g + 1) % 2)

        @pl.when(g > 1)
        def _():
            out_copy(g - 1).wait()

        if last:
            for piece in range(NS + N - 1):
                out_copy(g, piece).wait()

    @pl.when(g == 0)
    def _():
        z_ref[0] = 0
        body(True, False)
        wait_inputs(1)

    @pl.when(jnp.logical_and(g > 0, g < NH))
    def _():
        step(False)

    @pl.when(g == NH)
    def _():
        step(True)


@jax.jit
def pallas_standalone__mha_softmax__prompt_kernel(q: jax.Array, k: jax.Array, v: jax.Array):
    B, H, sq, d = q.shape
    assert sq == S and d == D and k.shape == q.shape and v.shape == q.shape
    NH = B * H
    qT, kT, vT = [jnp.swapaxes(x, 2, 3).reshape(NH, D, S) for x in (q, k, v)]
    oT = pl.pallas_call(
        _kernel,
        grid=(NH + 1,),
        in_specs=[pl.BlockSpec(memory_space=pl.ANY)] * 3,
        out_specs=pl.BlockSpec(memory_space=pl.ANY),
        out_shape=jax.ShapeDtypeStruct((NH, D, S), q.dtype),
        scratch_shapes=[pltpu.VMEM((2, 3, D, S), q.dtype), pltpu.VMEM((2, D, S), q.dtype),
                        pltpu.SMEM((1,), jnp.int32),
                        pltpu.VMEM((3 * LSZ, 128), U32), pltpu.VMEM((3 * LSZ, 128), U32),
                        pltpu.VMEM((2 * ASZ, 128), U32), pltpu.VMEM((ASZ + 64, 256), U32),
                        pltpu.VMEM((NT * HD, 128), U32),
                        pltpu.VMEM((NSTATE * 4 + 16, 8, 128), F32),
                        pltpu.SemaphoreType.DMA((5,)), pltpu.SemaphoreType.DMA((NS + N,))]
                       + [pltpu.VMEM((S + 8 + 8 * NGV, W), F32) for _ in range(NB)]
                       + [pltpu.VMEM((BROWS + 8, 256), U32) for _ in range(NBB)]
                       + [pltpu.VMEM((NP * HD + 8, 128), F32) for _ in range(2)],
        compiler_params=pltpu.CompilerParams(dimension_semantics=("arbitrary",),
                                             vmem_limit_bytes=100 * 1024 * 1024,
                                             disable_bounds_checks=True),
    )(qT, kT, vT)
    return jnp.swapaxes(oT.reshape(B, H, D, S), 2, 3)
```

```python
import bisect
import math

import jax
import jax.numpy as jnp
import jax.experimental.pallas as pl
import jax.experimental.pallas.tpu as pltpu

F32 = jnp.float32
BF16 = jnp.bfloat16
U32 = jnp.uint32

S = 2048
HD = 96
D = 2 * HD
W = 128
N = 4
HS = S // 2
NT = S // W
NS = NT // N
KB = S // N
NG = KB // 128
NB, NBB = 16, 4
NSTATE = 12
KEYS = ('m', 'e', 'M', 'l')

LAM = [1.0 / math.tan(math.pi * (i + 1) / (N + 1)) for i in range(N)]
PAIRS = [(i, j) for i in range(N) for j in range(i + 1, N)]
PRODS = []
for _i in range(N):
    for _j in range(_i + 1, N):
        PRODS += [('s', _i, _j), ('x', _i, _j), ('y', _i, _j)]
    PRODS += [('e', _i, _i), ('f', _i, _i)]
NP = len(PRODS)
PIDX = {p: k for k, p in enumerate(PRODS)}
SUBS = [('d', 0, 2), ('p', 0, 2), ('d', 1, 3), ('p', 1, 3), ('p', 0, 1), ('p', 0, 3), ('p', 1, 2), ('p', 2, 3)]
NSUB = len(SUBS)


def _sgn(i, j):
    return 1.0 if (i + j) % 2 == 1 else -1.0


CH = 208
GV = 4
SIZES = [CH] * (HS // CH) + [HS % CH]
NCH = len(SIZES)
OFFS = [sum(SIZES[:i]) for i in range(NCH)]
GPT = NP * NG
TOT = (3 * HS * NT + NS * GPT * HD) // 4
PER = TOT / NS
NCL = (KB // 16) * NSUB
NGVS = [-(-(sz // 8) // GV) for sz in SIZES]
GOFF = [sum(NGVS[:i]) for i in range(NCH)]
NGV = sum(NGVS)
NEC = -(-NGV // 8)
NCC = N * (HD // 8)
KPIECES = 8
VSUB = len(PAIRS) + 1
NV = NG * (HD // 16) * VSUB
QA = 512
PV0, PVN, PVN2 = 18, 5, 14


def _plan(m_ql=200, m_lp=150, m_pm=600, tail=300, espan=450, m_c=250, cspan=5000,
          kt=(600, 6000), vt=(3000, 16000)):
    lead_p = PER + m_pm
    lead_q = lead_p + PER + m_lp + espan + m_ql
    span = TOT - tail
    lp = int(math.ceil(lead_p / PER * NCL / NSUB)) * NSUB
    lq = int(math.ceil(lead_q / (PER / N) * NCH)) + 1
    nm = NS * GPT
    order, load = [], [0, 0, 0, 0]

    def put(n):
        u = min(range(4), key=lambda u: load[u])
        load[u] += n
        return load[u] - n

    mi = rows = 0
    for k in range(NT * NCH):
        sz = SIZES[(k + lq) % NCH]
        order.append(('q', k, max(put(sz) for _ in range(3)), sz))
        rows += sz
        while mi < nm and min(load) + HD // 2 <= sorted(load)[1]:
            order.append(('m', mi, put(HD), HD)); mi += 1
        while mi + 4 <= rows * nm / (NT * HS) + 2 and mi + 4 <= nm:
            for _ in range(4):
                order.append(('m', mi, put(HD), HD)); mi += 1
    while mi < nm:
        order.append(('m', mi, put(HD), HD)); mi += 1

    tasks = [((i + 0.5) * span / (NCL * NS), 'p', i + lp) for i in range(NCL * NS)]
    for kd, idx, s0, sz in order:
        if kd == 'q' and (idx + lq) % NCH == NCH - 1:
            n = (idx + lq) // NCH
            for u in range(NEC):
                t = s0 + sz + m_ql + u * espan / NEC
                tasks.append((t - span, 'e', (n - NT) * NEC + u) if t >= span else (t, 'e', n * NEC + u))
    le = min(ti for _, kd, ti in tasks if kd == 'e')
    tasks += [(T * PER + m_c + u * cspan / NCC, 'c', T * NCC + u) for T in range(NS) for u in range(NCC)]
    tasks += [(kt[0] + i * (kt[1] - kt[0]) / KPIECES, 'k', i) for i in range(KPIECES)]
    tasks += [(vt[0] + i * (vt[1] - vt[0]) / NV, 'v', i) for i in range(NV)]
    tasks.sort()

    cands = sorted((s + 8 * i, pos, i) for pos, (_, _, s, sz) in enumerate(order) for i in range(sz // 8))
    times = [c[0] for c in cands]
    after, cur = [[] for _ in order], 0
    for t, kd, idx in tasks:
        i = min(bisect.bisect_left(times, t), len(cands) - 1)
        _, pos, vr = min(cands[i:i + 4], key=lambda c: c[1])
        cur = max(cur, pos)
        after[cur].append((kd, idx, pos, vr))
    return order, after, lq, le, lp


ORDER, AFTER, LQ, LE, LP = _plan()
BROWS = (NP // 2) * (KB // 2)
ASZ = NP * (NG // 2) * (HD // 2)
LSZ = HS // 2


def _live_keys(n):
    qdone = max(0, min(NCH, LQ - n * NCH))
    edone = max(0, min(NEC, LE - n * NEC))
    pdone = max(0, min(NCL, LP - (n // N) * NCL))
    ks = []
    if qdone > 0 and edone < NEC: ks.append('m')
    if 0 < edone < NEC: ks.append('e')
    if edone == NEC and pdone < NCL: ks.append('M')
    if pdone > 0: ks.append('l')
    return ks


def _gate(x, *ms):
    cnd = x > jnp.inf
    return [jnp.where(cnd, x, m) for m in ms]


def _kernel(q_hbm, k_hbm, v_hbm, o_hbm, ibuf, obuf, z_ref, Lc, Ln, Ac, An, Qc, st_scr, isem, osem, *rest):
    S_refs, B_refs, R_refs = rest[:NB], rest[NB:NB + NBB], rest[NB + NBB:]
    NH = q_hbm.shape[0]
    scale = (D ** -0.5) * math.log2(math.e)
    g = pl.program_id(0)

    def in_copy(i, head, par, sem):
        return pltpu.make_async_copy((q_hbm, k_hbm, v_hbm)[i].at[head], ibuf.at[par, i], isem.at[sem])

    def prefetch(par):
        head = jnp.minimum(g + 1, NH - 1)
        for i in range(3):
            in_copy(i, head, par, 0).start()

    def wait_inputs(par):
        pltpu.make_async_copy(ibuf.at[par], ibuf.at[par], isem.at[0]).wait()

    def out_copy(step, piece=None):
        if piece is None:
            return pltpu.make_async_copy(obuf.at[step % 2], o_hbm.at[step - 1], osem.at[0])
        cols = pl.ds(piece * N * W, N * W) if piece < NS - 1 else pl.ds((piece + (NS - 1) * (N - 1)) * W, W)
        return pltpu.make_async_copy(obuf.at[step % 2, :, cols], o_hbm.at[step - 1, :, cols], osem.at[1 + piece])

    def body(first, last):
        z = z_ref[0]
        zb = pl.multiple_of(z * 8, 8)
        fence = lambda r: pl.ds(pl.multiple_of(r + z * 8, 8), 8)
        par = 0 if first else g % 2
        q_next, k_next, v_next = [ibuf.at[par, i] for i in range(3)]
        st = [dict() for _ in range(NT + NSTATE)]
        acc, res = {}, {}
        done = dict(k=0, q=set(), p=set(), m=set(), c=set())

        def kprep(c0, c1):
            a1, a2, a3 = [k_next[r:r + 64, c0:c1] for r in (0, 64, 128)]
            b1, b2, b3 = [k_next[r:r + 64, HS + c0:HS + c1] for r in (0, 64, 128)]
            d1 = (a2.astype(F32) - b2.astype(F32)).astype(BF16)
            d2 = (b1.astype(F32) - a1.astype(F32)).astype(BF16)
            for i, (x, y) in enumerate(((a1, b2), (d1, a3), (d2, b3))):
                Ln[pl.ds(zb + i * LSZ + c0 // 2, (c1 - c0) // 2), :] = pltpu.bitcast(
                    jnp.concatenate([x, y], axis=0).T, U32)

        def vprep(sb, xs):
            rows = [jnp.concatenate([xs[j * (HD // 16) + r] for j in range(NG)], axis=1) for r in range(HD // 16)]
            x = jnp.concatenate([y for y in rows for _ in range(2)], axis=0)
            ldf = lambda half, kb: v_next[half * HD:(half + 1) * HD, kb * KB:(kb + 1) * KB].astype(F32)

            def put_a(p, u):
                for jp in range(NG // 2):
                    ao = (PIDX[p] * (NG // 2) + jp) * (HD // 2)
                    An[ao:ao + HD // 2, :] = pltpu.bitcast(u[:, jp * 256:(jp + 1) * 256].astype(BF16), U32)

            if sb == len(PAIRS):
                for i in range(N):
                    a1, = _gate(x, ldf(0, i))
                    put_a(('e', i, i), a1)
                    put_a(('f', i, i), LAM[i] * a1 + ldf(1, i))
            else:
                i, jj = PAIRS[sb]
                d = LAM[i] - LAM[jj]
                a1i, a2i = _gate(x, ldf(0, i), ldf(1, i))
                a1j, a2j = ldf(0, jj), ldf(1, jj)
                u = a1i + a1j if _sgn(i, jj) > 0 else a1i - a1j
                w = a2i + a2j if _sgn(i, jj) > 0 else a2i - a2j
                xn = u * (LAM[jj] / d) + w * (1.0 / d)
                put_a(('x', i, jj), xn)
                put_a(('y', i, jj), u + xn)
                put_a(('s', i, jj), a1i + xn)

        def qcopy(n):
            Qc[pl.ds(zb + n * HD, HD), :] = pltpu.bitcast(q_next[:, n * W:(n + 1) * W], U32)

        def qk(n, ci):
            t, nxt = st[n], n >= NT
            assert first or n < NB or (n - NB) // N in done['p']
            if nxt:
                assert first or done['k'] == KPIECES
                if 'q' not in t:
                    t['q'] = q_next[:, (n - NT) * W:(n - NT + 1) * W]
                q = t['q']
            else:
                q = pltpu.bitcast(Qc[pl.ds(zb + n * HD, HD), :], BF16)
            r0, rows = OFFS[ci], SIZES[ci]
            lhs = lambda i: pltpu.bitcast((Ln if nxt else Lc)[pl.ds(zb + i * LSZ + r0 // 2, rows // 2), :], BF16)
            p3 = jnp.dot(lhs(0), q[0:128], preferred_element_type=F32)
            p1 = jnp.dot(lhs(1), q[64:192], preferred_element_type=F32)
            p2 = jnp.dot(lhs(2), jnp.concatenate([q[0:64], q[128:192]], axis=0), preferred_element_type=F32)
            sa = (p1 + p3) * scale
            sb = (p2 + p3) * scale
            Sr = S_refs[n % NB]
            Sr[r0:r0 + rows, :] = sa
            Sr[HS + r0:HS + r0 + rows, :] = sb
            sab = jnp.maximum(sa, sb).reshape(rows // 8, 8, W)
            for gi in range(NGVS[ci]):
                gm = sab[gi * GV:(gi + 1) * GV].max(axis=0)
                go = S + 8 + (GOFF[ci] + gi) * 8
                Sr[go:go + 8, :] = gm
                t['m'] = jnp.maximum(t['m'], gm) if 'm' in t else gm
            if ci == NCH - 1:
                t['m'] = jnp.broadcast_to(jnp.max(t['m'], axis=0, keepdims=True), (8, W))
                Sr[fence(S), :] = t['m']
                done['q'].add(n)
                if not nxt and not last:
                    qcopy(n)
            return p3

        def ecl(idx, x):
            n, u = divmod(idx, NEC)
            assert n in done['q']
            t = st[n]
            g0, g1 = u * 8, min(NGV, u * 8 + 8)
            s = S_refs[n % NB][S + 8 + g0 * 8:S + 8 + g1 * 8, :].reshape(g1 - g0, 8, W)
            m, = _gate(x, t['m'])
            e = jnp.exp2(s - m[None]).sum(axis=0)
            t['e'] = t['e'] + e if 'e' in t else e
            if u == NEC - 1:
                tot = jnp.sum(t.pop('e'), axis=0, keepdims=True)
                t['M'] = t.pop('m') + jnp.broadcast_to(jnp.log2(tot), (8, W))

        def pstage(T, s0, s1, xs):
            ns = s1 - s0
            Br = B_refs[T % NBB]
            assert first or T < NBB or (T - NBB) in done['m']

            def put_b(p, v):
                off, cb = (PIDX[p] // 2) * (KB // 2), (PIDX[p] % 2) * W
                Br[off + 8 * s0:off + 8 * s1, cb:cb + W] = pltpu.bitcast(v.reshape(16 * ns, W).astype(BF16), U32)

            rs, cs, cnt, ev = {}, {}, {}, {}
            for sb, (kd, i, j) in enumerate(SUBS):
                x = jnp.stack(xs[sb::NSUB])
                Ms = dict(zip((i, j), _gate(x, st[N * T + i]['M'][None], st[N * T + j]['M'][None])))

                def b(kb, q):
                    s = S_refs[(N * T + q) % NB][kb * KB + 16 * s0:kb * KB + 16 * s1, :].reshape(ns, 2, 8, W)
                    return jnp.exp2(s - Ms[q][:, None])

                if kd == 'd':
                    for q in (i, j):
                        rs[q] = cs[q] = b(q, q)
                        cnt[q] = 1
                else:
                    bij, bji = b(i, j), b(j, i)
                    upd = (lambda a, v: a - v) if _sgn(i, j) > 0 else (lambda a, v: a + v)
                    put_b(('x', i, j), bij)
                    put_b(('y', i, j), bji)
                    put_b(('s', i, j), bij - bji)
                    rs[i], rs[j] = upd(rs[i], bij), upd(rs[j], bji)
                    cs[i], cs[j] = upd(cs[i], bji), upd(cs[j], bij)
                    cnt[i] += 1
                    cnt[j] += 1
                for q in (i, j):
                    if cnt[q] == N // 2:
                        ev[q] = cs[q][:, 0] + cs[q][:, 1]
                        ev[q] = ev[q] + ev[q]
                    if cnt[q] == N:
                        put_b(('e', q, q), rs[q])
                        put_b(('f', q, q), cs[q])
            for q in range(N):
                t = st[N * T + q]
                od = cs[q][:, 0] + cs[q][:, 1]
                for s in range(ns):
                    t['l'] = (t['l'] + ev[q][s] if 'l' in t else ev[q][s]) - od[s]
            if s1 == KB // 16:
                Br[fence(BROWS), 0:W] = pltpu.bitcast(st[N * T]['M'], U32)
                for q in range(N):
                    t = st[N * T + q]
                    del t['M']
                    t['l'] = jnp.broadcast_to(1.0 / jnp.sum(t['l'], axis=0, keepdims=True), (8, W))
                done['p'].add(T)

        def mgroup(gi):
            T, r = divmod(gi, GPT)
            pi, j = divmod(r, NG)
            assert T in done['p'] and (j > 0 or T < 1 or (T - 2) in done['c'])
            a = Ac[pl.ds(zb + (j % 2) * ASZ + ((pi * NG + j) // 2) * (HD // 2), HD // 2), :]
            bo = (pi // 2) * (KB // 2) + j * 64
            b = B_refs[T % NBB][bo:bo + 64, (pi % 2) * W:(pi % 2 + 1) * W]
            oj = jnp.dot(pltpu.bitcast(a, BF16), pltpu.bitcast(b, BF16), preferred_element_type=F32)
            acc['o'] = oj if j == 0 else acc['o'] + oj
            if j == NG - 1:
                R_refs[T % 2][pi * HD:(pi + 1) * HD, :] = acc.pop('o')
                inline = last and T == NS - 1
                if pi == NP - 1:
                    done['m'].add(T)
                    if not inline:
                        R_refs[T % 2][fence(NP * HD), :] = oj[0:8]
                if inline and PRODS[pi][0] == 'f':
                    combine(T, PRODS[pi][1], oj)
            return oj

        def combine(T, q, x):
            assert T < 0 or T in done['m'] or (last and T == NS - 1)
            R = lambda *p: R_refs[T % 2][PIDX[p] * HD:(PIDX[p] + 1) * HD, :]
            add = lambda a, sg, v: a + v if sg > 0 else a - v
            others = ([(i, -1.0, R('x', i, q)) for i in range(q)]
                      + [(jj, _sgn(q, jj), R('y', q, jj)) for jj in range(q + 1, N)])
            gq, = _gate(x, R('e', q, q))
            for jj in range(q + 1, N):
                gq = add(add(gq, _sgn(q, jj), R('s', q, jj)), -_sgn(q, jj), R('x', q, jj))
            for i in range(q):
                gq = (gq + R('y', i, q)) + R('s', i, q)
            c1 = gq
            c2 = R('f', q, q) - LAM[q] * gq
            for t_, sg, v in others:
                c1 = add(c1, sg, v)
                c2 = c2 - (sg * LAM[t_]) * v
            if T < 0:
                linv, ob = st_scr[NSTATE * 4 + q], obuf.at[(g - 1) % 2]
            else:
                linv, ob = st[N * T + q]['l'], obuf.at[g % 2]
            q0 = (N * (T % NS) + q) * W
            for half, cc in enumerate((c1, c2)):
                cc = (cc.reshape(HD // 8, 8, W) * linv[None]).reshape(HD, W)
                ob[half * HD:(half + 1) * HD, q0:q0 + W] = cc.astype(ob.dtype)
            if q == N - 1:
                done['c'].add(T)
                if T < 0:
                    @pl.when(g > 1)
                    def _():
                        out_copy(g - 1).start()
                elif last and T < NS - 1:
                    out_copy(g, T).start()
            if last and T == NS - 1:
                out_copy(g, T + q).start()

        pend = dict(p=[], c=[], v={})

        def flush_p(ti):
            T, k = divmod(ti, NCL)
            s1 = k // NSUB + 1
            pstage(T, s1 - len(pend['p']) // NSUB, s1, pend['p'])
            pend['p'] = []

        def pcl(ti, x):
            pend['p'].append(x)
            pend['pi'] = ti
            if ti % NCL == NCL - 1:
                flush_p(ti)

        def ccl(ti, x):
            pend['c'].append(x)
            if len(pend['c']) == HD // 8:
                T, u = divmod(ti, NCC)
                combine(T - 1, u // (HD // 8), jnp.concatenate(pend['c'], axis=0))
                pend['c'] = []

        def vcl(ti, x):
            pend['v'][ti] = x
            if ti >= NV - VSUB:
                vprep(ti % VSUB, [pend['v'][p * VSUB + ti % VSUB] for p in range(NV // VSUB)])

        if first:
            qa = pltpu.make_async_copy(q_hbm.at[0, :, 0:QA], ibuf.at[0, 0, :, 0:QA], isem.at[1])
            qb = pltpu.make_async_copy(q_hbm.at[0, :, QA:S], ibuf.at[0, 0, :, QA:S], isem.at[4])
            in_copy(1, 0, 0, 2).start()
            qa.start()
            in_copy(2, 0, 0, 3).start()
            qb.start()
            R_refs[(NS - 1) % 2][0:NP * HD, :] = jnp.zeros((NP * HD, W), F32)
            for q in range(N):
                st_scr[NSTATE * 4 + q] = jnp.zeros((8, W), F32)
            in_copy(1, 0, 0, 2).wait()
            qa.wait()
            kprep(0, HS)
        else:
            Lc[pl.ds(zb, 3 * LSZ), :] = Ln[pl.ds(zb, 3 * LSZ), :]
            for i in range(2):
                Ac[pl.ds(zb + i * ASZ, ASZ), :] = An[0:ASZ, i * W:(i + 1) * W]
            for n in range(NSTATE):
                for key in _live_keys(n):
                    st[n][key] = st_scr[n * 4 + KEYS.index(key)]
                if LQ >= (n + 1) * NCH: done['q'].add(n)
                if LP >= (n // N + 1) * NCL: done['p'].add(n // N)

        pw = HS // KPIECES
        run = dict(e=ecl, p=pcl, c=ccl, v=vcl)

        def active(pos):
            kd, idx = ORDER[pos][0:2]
            if kd == 'm': return not first
            n = (idx + LQ) // NCH
            return (not first or n >= NT) and (not last or n < NT)

        def wanted(tk, ti):
            lim = NCL * NS if tk == 'p' else NT * NEC
            if first: return tk not in 'kvc' and ti >= lim
            if last: return tk == 'c' or (tk not in 'kv' and ti < lim)
            return True

        acts = [pos for pos in range(len(ORDER)) if active(pos)]
        nq, vdone = 0, 0
        for ai, pos in enumerate(acts):
            kd, idx = ORDER[pos][0:2]
            res[pos] = qk(*divmod(idx + LQ, NCH)) if kd == 'q' else mgroup(idx)
            end = acts[ai + 1] if ai + 1 < len(acts) else len(ORDER)
            todo = [t for p2 in range(pos, end) for t in AFTER[p2] if wanted(t[0], t[1])]
            if first:
                nq += 1
                if nq == PV0:
                    assert nq <= (QA // W) * NCH
                    in_copy(2, 0, 0, 3).wait()
                    qb.wait()
                    prefetch(1)
                if nq == PV0 + 1:
                    for n2 in range(LQ // NCH, NT):
                        qcopy(n2)
                if nq > PV0:
                    nv = min(NV - vdone, PVN if todo else PVN2)
                    vs = [('v', vdone + u, None, 0) for u in range(nv)]
                    vdone += nv
                    mix = sorted([((i + 0.5) / len(todo), t) for i, t in enumerate(todo)]
                                 + [((i + 0.25) / nv, t) for i, t in enumerate(vs)], key=lambda a: a[0])
                    todo = [t for _, t in mix]
            nvr = res[pos].shape[0] // 8
            for i, (tk, ti, tpos, vr) in enumerate(todo):
                if first or tpos not in res:
                    tpos, vr = pos, (i * nvr) // len(todo)
                x = res[tpos][8 * vr:8 * vr + 8]
                if tk == 'k':
                    kprep(ti * pw, (ti + 1) * pw)
                    done['k'] += 1
                else:
                    run[tk](ti, x)
        if pend['p']:
            flush_p(pend['pi'])
        assert not pend['c'] and (not first or vdone == NV)
        if not last:
            if not first:
                for q in range(N):
                    st_scr[NSTATE * 4 + q] = st[NT - N + q]['l']
            for n in range(NSTATE):
                assert sorted(k for k in st[NT + n] if k != 'q') == sorted(_live_keys(n))
                for key in _live_keys(n):
                    st_scr[n * 4 + KEYS.index(key)] = st[NT + n][key]

    def step(last):
        if not last:
            prefetch((g + 1) % 2)
        body(False, last)
        if not last:
            wait_inputs((g + 1) % 2)

        @pl.when(g > 1)
        def _():
            out_copy(g - 1).wait()

        if last:
            for piece in range(NS + N - 1):
                out_copy(g, piece).wait()

    @pl.when(g == 0)
    def _():
        z_ref[0] = 0
        body(True, False)
        wait_inputs(1)

    @pl.when(jnp.logical_and(g > 0, g < NH))
    def _():
        step(False)

    @pl.when(g == NH)
    def _():
        step(True)


@jax.jit
def pallas_standalone__mha_softmax__prompt_kernel(q: jax.Array, k: jax.Array, v: jax.Array):
    B, H, sq, d = q.shape
    assert sq == S and d == D and k.shape == q.shape and v.shape == q.shape
    NH = B * H
    qT, kT, vT = [jnp.swapaxes(x, 2, 3).reshape(NH, D, S) for x in (q, k, v)]
    oT = pl.pallas_call(
        _kernel,
        grid=(NH + 1,),
        in_specs=[pl.BlockSpec(memory_space=pl.ANY)] * 3,
        out_specs=pl.BlockSpec(memory_space=pl.ANY),
        out_shape=jax.ShapeDtypeStruct((NH, D, S), q.dtype),
        scratch_shapes=[pltpu.VMEM((2, 3, D, S), q.dtype), pltpu.VMEM((2, D, S), q.dtype),
                        pltpu.SMEM((1,), jnp.int32),
                        pltpu.VMEM((3 * LSZ, 128), U32), pltpu.VMEM((3 * LSZ, 128), U32),
                        pltpu.VMEM((2 * ASZ, 128), U32), pltpu.VMEM((ASZ + 64, 256), U32),
                        pltpu.VMEM((NT * HD, 128), U32),
                        pltpu.VMEM((NSTATE * 4 + 16, 8, 128), F32),
                        pltpu.SemaphoreType.DMA((5,)), pltpu.SemaphoreType.DMA((NS + N,))]
                       + [pltpu.VMEM((S + 8 + 8 * NGV, W), F32) for _ in range(NB)]
                       + [pltpu.VMEM((BROWS + 8, 256), U32) for _ in range(NBB)]
                       + [pltpu.VMEM((NP * HD + 8, 128), F32) for _ in range(2)],
        compiler_params=pltpu.CompilerParams(dimension_semantics=("arbitrary",),
                                             vmem_limit_bytes=100 * 1024 * 1024,
                                             disable_bounds_checks=True),
    )(qT, kT, vT)
    return jnp.swapaxes(oT.reshape(B, H, D, S), 2, 3)
```

```python
import bisect
import math

import jax
import jax.numpy as jnp
import jax.experimental.pallas as pl
import jax.experimental.pallas.tpu as pltpu

F32 = jnp.float32
BF16 = jnp.bfloat16
U32 = jnp.uint32

S = 2048
HD = 96
D = 2 * HD
W = 128
N = 4
HS = S // 2
NT = S // W
NS = NT // N
KB = S // N
NG = KB // 128
NB, NBB = 16, 4
NSTATE = 12
KEYS = ('m', 'e', 'M', 'l')

LAM = [1.0 / math.tan(math.pi * (i + 1) / (N + 1)) for i in range(N)]
PAIRS = [(i, j) for i in range(N) for j in range(i + 1, N)]
PRODS = []
for _i in range(N):
    for _j in range(_i + 1, N):
        PRODS += [('s', _i, _j), ('x', _i, _j), ('y', _i, _j)]
    PRODS += [('e', _i, _i), ('f', _i, _i)]
NP = len(PRODS)
PIDX = {p: k for k, p in enumerate(PRODS)}
SUBS = [('d', 0, 2), ('p', 0, 2), ('d', 1, 3), ('p', 1, 3), ('p', 0, 1), ('p', 0, 3), ('p', 1, 2), ('p', 2, 3)]
NSUB = len(SUBS)


def _sgn(i, j):
    return 1.0 if (i + j) % 2 == 1 else -1.0


CH = 208
GV = 4
SIZES = [CH] * (HS // CH) + [HS % CH]
NCH = len(SIZES)
OFFS = [sum(SIZES[:i]) for i in range(NCH)]
GPT = NP * NG
TOT = (3 * HS * NT + NS * GPT * HD) // 4
PER = TOT / NS
NPC = 2 * NSUB
NCL = (KB // 16) * NPC
NGVS = [-(-(sz // 8) // GV) for sz in SIZES]
GOFF = [sum(NGVS[:i]) for i in range(NCH)]
NGV = sum(NGVS)
EG = 4
NEC = -(-NGV // EG)
NCC = N * (HD // 8)
KPIECES = 8
VSUB = len(PAIRS) + 1
NV = NG * (HD // 8) * VSUB
QA = 384
PV0, PVN, PVN2 = 15, 7, 26


def _plan(m_ql=150, m_lp=150, m_pm=650, tail=300, espan=450, m_c=250, cspan=4500,
          kt=(600, 6000), vt=(500, 21000), ww=0.5, alpha=0.25):
    lead_p = PER + m_pm
    lead_q = lead_p + PER + m_lp + espan + m_ql
    span = TOT - tail
    lp = int(math.ceil(lead_p / PER * NCL / NPC)) * NPC
    lq = int(math.ceil(lead_q / (PER / N) * NCH)) + 1
    nm = NS * GPT
    order, load = [], [0, 0, 0, 0]

    def put(n):
        u = min(range(4), key=lambda u: load[u])
        load[u] += n
        return load[u] - n

    mi = rows = 0
    for k in range(NT * NCH):
        sz = SIZES[(k + lq) % NCH]
        order.append(('q', k, max(put(sz) for _ in range(3)), sz))
        rows += sz
        while mi < nm and min(load) + HD // 2 <= sorted(load)[1]:
            order.append(('m', mi, put(HD), HD)); mi += 1
        while mi + 4 <= rows * nm / (NT * HS) + 2 and mi + 4 <= nm:
            for _ in range(4):
                order.append(('m', mi, put(HD), HD)); mi += 1
    while mi < nm:
        order.append(('m', mi, put(HD), HD)); mi += 1

    wts, cnt = [], {}
    for kd, i, j in SUBS:
        if kd == 'd':
            cnt[i] = cnt[j] = 1
            wts += [6.0, 6.0]
        else:
            cnt[i] += 1
            cnt[j] += 1
            extra = sum({N // 2: 1.5, N: 3.0}.get(cnt[q], 0.0) for q in (i, j))
            wts += [12.0 + extra, 16.0 + extra]
    wts = [(1 - ww) + ww * w * len(wts) / sum(wts) for w in wts]
    cap = [1.0] * (TOT // 8 + 64)
    for kd, _, s0, sz in order:
        if kd == 'q':
            cap[s0 // 8:(s0 + sz) // 8] = [1.0 - alpha] * (sz // 8)
    cum = [0.0]
    for t in range(span // 8):
        cum.append(cum[-1] + cap[t])
    tasks, w0 = [], 0.5
    for i in range(NCL * NS):
        y = w0 / (NCL * NS) * cum[-1]
        k = min(bisect.bisect_right(cum, y) - 1, len(cum) - 2)
        tasks.append((8 * (k + (y - cum[k]) / cap[k]), 'p', i + lp))
        w0 += wts[i % NPC]
    for kd, idx, s0, sz in order:
        if kd == 'q' and (idx + lq) % NCH == NCH - 1:
            n = (idx + lq) // NCH
            for u in range(NEC):
                t = s0 + sz + m_ql + u * espan / NEC
                tasks.append((t - span, 'e', (n - NT) * NEC + u) if t >= span else (t, 'e', n * NEC + u))
    le = min(ti for _, kd, ti in tasks if kd == 'e')
    tasks += [(T * PER + m_c + u * cspan / NCC, 'c', T * NCC + u) for T in range(NS) for u in range(NCC)]
    tasks += [(kt[0] + i * (kt[1] - kt[0]) / KPIECES, 'k', i) for i in range(KPIECES)]
    tasks += [(vt[0] + i * (vt[1] - vt[0]) / NV, 'v', i) for i in range(NV)]
    tasks.sort()

    cands = sorted((s + 8 * i, pos, i) for pos, (_, _, s, sz) in enumerate(order) for i in range(sz // 8))
    times = [c[0] for c in cands]
    after, cur = [[] for _ in order], 0
    for t, kd, idx in tasks:
        i = min(bisect.bisect_left(times, t), len(cands) - 1)
        _, pos, vr = min(cands[i:i + 4], key=lambda c: (order[c[1]][0] != 'm', c[1]))
        cur = max(cur, pos)
        after[cur].append((kd, idx, pos, vr))
    return order, after, lq, le, lp


ORDER, AFTER, LQ, LE, LP = _plan()
BROWS = (NP // 2) * (KB // 2)
ASZ = NP * (NG // 2) * (HD // 2)
LSZ = HS // 2


def _live_keys(n):
    qdone = max(0, min(NCH, LQ - n * NCH))
    edone = max(0, min(NEC, LE - n * NEC))
    pdone = max(0, min(NCL, LP - (n // N) * NCL))
    ks = []
    if qdone > 0 and edone < NEC: ks.append('m')
    if 0 < edone < NEC: ks.append('e')
    if edone == NEC and pdone < NCL: ks.append('M')
    if pdone > 0: ks.append('l')
    return ks


def _gate(x, *ms):
    cnd = x > jnp.inf
    return [jnp.where(cnd, x, m) for m in ms]


def _kernel(q_hbm, k_hbm, v_hbm, o_hbm, ibuf, obuf, z_ref, Lc, Ln, Ac, An, Qc, st_scr, isem, osem, *rest):
    S_refs, B_refs, R_refs = rest[:NB], rest[NB:NB + NBB], rest[NB + NBB:]
    NH = q_hbm.shape[0]
    scale = (D ** -0.5) * math.log2(math.e)
    g = pl.program_id(0)

    def in_copy(i, head, par, sem):
        return pltpu.make_async_copy((q_hbm, k_hbm, v_hbm)[i].at[head], ibuf.at[par, i], isem.at[sem])

    def prefetch(par):
        head = jnp.minimum(g + 1, NH - 1)
        for i in range(3):
            in_copy(i, head, par, 0).start()

    def wait_inputs(par):
        pltpu.make_async_copy(ibuf.at[par], ibuf.at[par], isem.at[0]).wait()

    def out_copy(step, piece=None):
        if piece is None:
            return pltpu.make_async_copy(obuf.at[step % 2], o_hbm.at[step - 1], osem.at[0])
        cols = pl.ds(piece * N * W, N * W) if piece < NS - 1 else pl.ds((piece + (NS - 1) * (N - 1)) * W, W)
        return pltpu.make_async_copy(obuf.at[step % 2, :, cols], o_hbm.at[step - 1, :, cols], osem.at[1 + piece])

    def body(first, last):
        z = z_ref[0]
        zb = pl.multiple_of(z * 8, 8)
        fence = lambda r: pl.ds(pl.multiple_of(r + z * 8, 8), 8)
        par = 0 if first else g % 2
        q_next, k_next, v_next = [ibuf.at[par, i] for i in range(3)]
        st = [dict() for _ in range(NT + NSTATE)]
        acc, res = {}, {}
        done = dict(k=0, q=set(), p=set(), m=set(), c=set())

        def kprep(c0, c1):
            a1, a2, a3 = [k_next[r:r + 64, c0:c1] for r in (0, 64, 128)]
            b1, b2, b3 = [k_next[r:r + 64, HS + c0:HS + c1] for r in (0, 64, 128)]
            d1 = (a2.astype(F32) - b2.astype(F32)).astype(BF16)
            d2 = (b1.astype(F32) - a1.astype(F32)).astype(BF16)
            for i, (x, y) in enumerate(((a1, b2), (d1, a3), (d2, b3))):
                Ln[pl.ds(zb + i * LSZ + c0 // 2, (c1 - c0) // 2), :] = pltpu.bitcast(
                    jnp.concatenate([x, y], axis=0).T, U32)

        def vprep(sb, xs):
            x = jnp.concatenate([jnp.concatenate(xs[r::HD // 8], axis=1) for r in range(HD // 8)], axis=0)
            ldf = lambda half, kb: v_next[half * HD:(half + 1) * HD, kb * KB:(kb + 1) * KB].astype(F32)

            def put_a(p, u):
                for jp in range(NG // 2):
                    ao = (PIDX[p] * (NG // 2) + jp) * (HD // 2)
                    An[ao:ao + HD // 2, :] = pltpu.bitcast(u[:, jp * 256:(jp + 1) * 256].astype(BF16), U32)

            if sb == len(PAIRS):
                for i in range(N):
                    a1, = _gate(x, ldf(0, i))
                    put_a(('e', i, i), a1)
                    put_a(('f', i, i), LAM[i] * a1 + ldf(1, i))
            else:
                i, jj = PAIRS[sb]
                d = LAM[i] - LAM[jj]
                a1i, a2i = _gate(x, ldf(0, i), ldf(1, i))
                a1j, a2j = ldf(0, jj), ldf(1, jj)
                u = a1i + a1j if _sgn(i, jj) > 0 else a1i - a1j
                w = a2i + a2j if _sgn(i, jj) > 0 else a2i - a2j
                xn = u * (LAM[jj] / d) + w * (1.0 / d)
                put_a(('x', i, jj), xn)
                put_a(('y', i, jj), u + xn)
                put_a(('s', i, jj), a1i + xn)

        def qcopy(n):
            Qc[pl.ds(zb + n * HD, HD), :] = pltpu.bitcast(q_next[:, n * W:(n + 1) * W], U32)

        def qk(n, ci):
            t, nxt = st[n], n >= NT
            assert first or n < NB or (n - NB) // N in done['p']
            if nxt:
                assert first or done['k'] == KPIECES
                if 'q' not in t:
                    t['q'] = q_next[:, (n - NT) * W:(n - NT + 1) * W]
                q = t['q']
            else:
                q = pltpu.bitcast(Qc[pl.ds(zb + n * HD, HD), :], BF16)
            r0, rows = OFFS[ci], SIZES[ci]
            lhs = lambda i: pltpu.bitcast((Ln if nxt else Lc)[pl.ds(zb + i * LSZ + r0 // 2, rows // 2), :], BF16)
            p3 = jnp.dot(lhs(0), q[0:128], preferred_element_type=F32)
            p1 = jnp.dot(lhs(1), q[64:192], preferred_element_type=F32)
            p2 = jnp.dot(lhs(2), jnp.concatenate([q[0:64], q[128:192]], axis=0), preferred_element_type=F32)
            sa = (p1 + p3) * scale
            sb = (p2 + p3) * scale
            Sr = S_refs[n % NB]
            Sr[r0:r0 + rows, :] = sa
            Sr[HS + r0:HS + r0 + rows, :] = sb
            sab = jnp.maximum(sa, sb).reshape(rows // 8, 8, W)
            for gi in range(NGVS[ci]):
                gm = sab[gi * GV:(gi + 1) * GV].max(axis=0)
                go = S + 8 + (GOFF[ci] + gi) * 8
                Sr[go:go + 8, :] = gm
                t['m'] = jnp.maximum(t['m'], gm) if 'm' in t else gm
            if ci == NCH - 1:
                t['m'] = jnp.broadcast_to(jnp.max(t['m'], axis=0, keepdims=True), (8, W))
                Sr[fence(S), :] = t['m']
                done['q'].add(n)
                if not nxt and not last:
                    qcopy(n)
            return p3

        def ecl(idx, x):
            n, u = divmod(idx, NEC)
            assert n in done['q']
            t = st[n]
            g0, g1 = u * EG, min(NGV, u * EG + EG)
            s = S_refs[n % NB][S + 8 + g0 * 8:S + 8 + g1 * 8, :].reshape(g1 - g0, 8, W)
            m, = _gate(x, t['m'])
            e = jnp.exp2(s - m[None]).sum(axis=0)
            t['e'] = t['e'] + e if 'e' in t else e
            if u == NEC - 1:
                tot = jnp.sum(t.pop('e'), axis=0, keepdims=True)
                t['M'] = t.pop('m') + jnp.broadcast_to(jnp.log2(tot), (8, W))

        def pstage(T, s0, s1, xs):
            ns = s1 - s0
            Br = B_refs[T % NBB]
            assert first or T < NBB or (T - NBB) in done['m']

            def put_b(p, v):
                off, cb = (PIDX[p] // 2) * (KB // 2), (PIDX[p] % 2) * W
                Br[off + 8 * s0:off + 8 * s1, cb:cb + W] = pltpu.bitcast(v.reshape(16 * ns, W).astype(BF16), U32)

            rs, cs, cnt, ev = {}, {}, {}, {}
            for sb, (kd, i, j) in enumerate(SUBS):
                Ms = {q: _gate(jnp.stack(xs[2 * sb + hh::NPC]), st[N * T + q]['M'][None])[0]
                      for hh, q in enumerate((j, i))}

                def b(kb, q):
                    s = S_refs[(N * T + q) % NB][kb * KB + 16 * s0:kb * KB + 16 * s1, :].reshape(ns, 2, 8, W)
                    return jnp.exp2(s - Ms[q][:, None])

                if kd == 'd':
                    for q in (i, j):
                        rs[q] = cs[q] = b(q, q)
                        cnt[q] = 1
                else:
                    bij, bji = b(i, j), b(j, i)
                    upd = (lambda a, v: a - v) if _sgn(i, j) > 0 else (lambda a, v: a + v)
                    put_b(('x', i, j), bij)
                    put_b(('y', i, j), bji)
                    put_b(('s', i, j), bij - bji)
                    rs[i], rs[j] = upd(rs[i], bij), upd(rs[j], bji)
                    cs[i], cs[j] = upd(cs[i], bji), upd(cs[j], bij)
                    cnt[i] += 1
                    cnt[j] += 1
                for q in (i, j):
                    if cnt[q] == N // 2:
                        ev[q] = cs[q][:, 0] + cs[q][:, 1]
                        ev[q] = ev[q] + ev[q]
                    if cnt[q] == N:
                        put_b(('e', q, q), rs[q])
                        put_b(('f', q, q), cs[q])
            for q in range(N):
                t = st[N * T + q]
                od = cs[q][:, 0] + cs[q][:, 1]
                for s in range(ns):
                    t['l'] = (t['l'] + ev[q][s] if 'l' in t else ev[q][s]) - od[s]
            if s1 == KB // 16:
                Br[fence(BROWS), 0:W] = pltpu.bitcast(st[N * T]['M'], U32)
                for q in range(N):
                    t = st[N * T + q]
                    del t['M']
                    t['l'] = jnp.broadcast_to(1.0 / jnp.sum(t['l'], axis=0, keepdims=True), (8, W))
                done['p'].add(T)

        def mgroup(gi):
            T, r = divmod(gi, GPT)
            pi, j = divmod(r, NG)
            assert T in done['p'] and (j > 0 or T < 1 or (T - 2) in done['c'])
            a = Ac[pl.ds(zb + (j % 2) * ASZ + ((pi * NG + j) // 2) * (HD // 2), HD // 2), :]
            bo = (pi // 2) * (KB // 2) + j * 64
            b = B_refs[T % NBB][bo:bo + 64, (pi % 2) * W:(pi % 2 + 1) * W]
            oj = jnp.dot(pltpu.bitcast(a, BF16), pltpu.bitcast(b, BF16), preferred_element_type=F32)
            acc['o'] = oj if j == 0 else acc['o'] + oj
            if j == NG - 1:
                R_refs[T % 2][pi * HD:(pi + 1) * HD, :] = acc.pop('o')
                inline = last and T == NS - 1
                if pi == NP - 1:
                    done['m'].add(T)
                    if not inline:
                        R_refs[T % 2][fence(NP * HD), :] = oj[0:8]
                if inline and PRODS[pi][0] == 'f':
                    combine(T, PRODS[pi][1], oj)
            return oj

        def combine(T, q, x):
            assert T < 0 or T in done['m'] or (last and T == NS - 1)
            R = lambda *p: R_refs[T % 2][PIDX[p] * HD:(PIDX[p] + 1) * HD, :]
            add = lambda a, sg, v: a + v if sg > 0 else a - v
            others = ([(i, -1.0, R('x', i, q)) for i in range(q)]
                      + [(jj, _sgn(q, jj), R('y', q, jj)) for jj in range(q + 1, N)])
            gq, = _gate(x, R('e', q, q))
            for jj in range(q + 1, N):
                gq = add(add(gq, _sgn(q, jj), R('s', q, jj)), -_sgn(q, jj), R('x', q, jj))
            for i in range(q):
                gq = (gq + R('y', i, q)) + R('s', i, q)
            c1 = gq
            c2 = R('f', q, q) - LAM[q] * gq
            for t_, sg, v in others:
                c1 = add(c1, sg, v)
                c2 = c2 - (sg * LAM[t_]) * v
            if T < 0:
                linv, ob = st_scr[NSTATE * 4 + q], obuf.at[(g - 1) % 2]
            else:
                linv, ob = st[N * T + q]['l'], obuf.at[g % 2]
            q0 = (N * (T % NS) + q) * W
            for half, cc in enumerate((c1, c2)):
                cc = (cc.reshape(HD // 8, 8, W) * linv[None]).reshape(HD, W)
                ob[half * HD:(half + 1) * HD, q0:q0 + W] = cc.astype(ob.dtype)
            if q == N - 1:
                done['c'].add(T)
                if T < 0:
                    @pl.when(g > 1)
                    def _():
                        out_copy(g - 1).start()
                elif last and T < NS - 1:
                    out_copy(g, T).start()
            if last and T == NS - 1:
                out_copy(g, T + q).start()

        pend = dict(p=[], c=[], v={})

        def flush_p(ti):
            T, k = divmod(ti, NCL)
            s1 = k // NPC + 1
            pstage(T, s1 - len(pend['p']) // NPC, s1, pend['p'])
            pend['p'] = []

        def pcl(ti, x):
            pend['p'].append(x)
            pend['pi'] = ti
            if ti % NCL == NCL - 1:
                flush_p(ti)

        def ccl(ti, x):
            pend['c'].append(x)
            if len(pend['c']) == HD // 8:
                T, u = divmod(ti, NCC)
                combine(T - 1, u // (HD // 8), jnp.concatenate(pend['c'], axis=0))
                pend['c'] = []

        def vcl(ti, x):
            pend['v'][ti] = x
            if ti >= NV - 2 * VSUB and ti % 2 == 1:
                sb = (ti // 2) % VSUB
                vprep(sb, [pend['v'][((p // 2) * VSUB + sb) * 2 + p % 2] for p in range(NV // VSUB)])

        if first:
            qa = pltpu.make_async_copy(q_hbm.at[0, :, 0:QA], ibuf.at[0, 0, :, 0:QA], isem.at[1])
            qb = pltpu.make_async_copy(q_hbm.at[0, :, QA:S], ibuf.at[0, 0, :, QA:S], isem.at[4])
            in_copy(1, 0, 0, 2).start()
            qa.start()
            in_copy(2, 0, 0, 3).start()
            qb.start()
            R_refs[(NS - 1) % 2][0:NP * HD, :] = jnp.zeros((NP * HD, W), F32)
            for q in range(N):
                st_scr[NSTATE * 4 + q] = jnp.zeros((8, W), F32)
            in_copy(1, 0, 0, 2).wait()
            qa.wait()
            kprep(0, HS)
        else:
            Lc[pl.ds(zb, 3 * LSZ), :] = Ln[pl.ds(zb, 3 * LSZ), :]
            for i in range(2):
                Ac[pl.ds(zb + i * ASZ, ASZ), :] = An[0:ASZ, i * W:(i + 1) * W]
            for n in range(NSTATE):
                for key in _live_keys(n):
                    st[n][key] = st_scr[n * 4 + KEYS.index(key)]
                if LQ >= (n + 1) * NCH: done['q'].add(n)
                if LP >= (n // N + 1) * NCL: done['p'].add(n // N)

        pw = HS // KPIECES
        run = dict(e=ecl, p=pcl, c=ccl, v=vcl)

        def active(pos):
            kd, idx = ORDER[pos][0:2]
            if kd == 'm': return not first
            n = (idx + LQ) // NCH
            return (not first or n >= NT) and (not last or n < NT)

        def wanted(tk, ti):
            lim = NCL * NS if tk == 'p' else NT * NEC
            if first: return tk not in 'kvc' and ti >= lim
            if last: return tk == 'c' or (tk not in 'kv' and ti < lim)
            return True

        acts = [pos for pos in range(len(ORDER)) if active(pos)]
        nq, vdone = 0, 0
        for ai, pos in enumerate(acts):
            kd, idx = ORDER[pos][0:2]
            res[pos] = qk(*divmod(idx + LQ, NCH)) if kd == 'q' else mgroup(idx)
            end = acts[ai + 1] if ai + 1 < len(acts) else len(ORDER)
            todo = [t for p2 in range(pos, end) for t in AFTER[p2] if wanted(t[0], t[1])]
            if first:
                nq += 1
                if nq == PV0:
                    assert nq <= (QA // W) * NCH
                    in_copy(2, 0, 0, 3).wait()
                    qb.wait()
                    prefetch(1)
                if nq == PV0 + 1:
                    for n2 in range(LQ // NCH, NT):
                        qcopy(n2)
                if nq > PV0:
                    nv = min(NV - vdone, PVN if any(t[0] == 'p' for t in todo) else PVN2)
                    vs = [('v', vdone + u, None, 0) for u in range(nv)]
                    vdone += nv
                    mix = sorted([((i + 0.5) / len(todo), t) for i, t in enumerate(todo)]
                                 + [((i + 0.25) / nv, t) for i, t in enumerate(vs)], key=lambda a: a[0])
                    todo = [t for _, t in mix]
            nvr = res[pos].shape[0] // 8
            for i, (tk, ti, tpos, vr) in enumerate(todo):
                if first or tpos not in res:
                    tpos, vr = pos, (i * nvr) // len(todo)
                x = res[tpos][8 * vr:8 * vr + 8]
                if tk == 'k':
                    kprep(ti * pw, (ti + 1) * pw)
                    done['k'] += 1
                else:
                    run[tk](ti, x)
        if pend['p']:
            flush_p(pend['pi'])
        assert not pend['c'] and (not first or vdone == NV)
        if not last:
            if not first:
                for q in range(N):
                    st_scr[NSTATE * 4 + q] = st[NT - N + q]['l']
            for n in range(NSTATE):
                assert sorted(k for k in st[NT + n] if k != 'q') == sorted(_live_keys(n))
                for key in _live_keys(n):
                    st_scr[n * 4 + KEYS.index(key)] = st[NT + n][key]

    def step(last):
        if not last:
            prefetch((g + 1) % 2)
        body(False, last)
        if not last:
            wait_inputs((g + 1) % 2)

        @pl.when(g > 1)
        def _():
            out_copy(g - 1).wait()

        if last:
            for piece in range(NS + N - 1):
                out_copy(g, piece).wait()

    @pl.when(g == 0)
    def _():
        z_ref[0] = 0
        body(True, False)
        wait_inputs(1)

    @pl.when(jnp.logical_and(g > 0, g < NH))
    def _():
        step(False)

    @pl.when(g == NH)
    def _():
        step(True)


@jax.jit
def pallas_standalone__mha_softmax__prompt_kernel(q: jax.Array, k: jax.Array, v: jax.Array):
    B, H, sq, d = q.shape
    assert sq == S and d == D and k.shape == q.shape and v.shape == q.shape
    NH = B * H
    qT, kT, vT = [jnp.swapaxes(x, 2, 3).reshape(NH, D, S) for x in (q, k, v)]
    oT = pl.pallas_call(
        _kernel,
        grid=(NH + 1,),
        in_specs=[pl.BlockSpec(memory_space=pl.ANY)] * 3,
        out_specs=pl.BlockSpec(memory_space=pl.ANY),
        out_shape=jax.ShapeDtypeStruct((NH, D, S), q.dtype),
        scratch_shapes=[pltpu.VMEM((2, 3, D, S), q.dtype), pltpu.VMEM((2, D, S), q.dtype),
                        pltpu.SMEM((1,), jnp.int32),
                        pltpu.VMEM((3 * LSZ, 128), U32), pltpu.VMEM((3 * LSZ, 128), U32),
                        pltpu.VMEM((2 * ASZ, 128), U32), pltpu.VMEM((ASZ + 64, 256), U32),
                        pltpu.VMEM((NT * HD, 128), U32),
                        pltpu.VMEM((NSTATE * 4 + 16, 8, 128), F32),
                        pltpu.SemaphoreType.DMA((5,)), pltpu.SemaphoreType.DMA((NS + N,))]
                       + [pltpu.VMEM((S + 8 + 8 * NGV, W), F32) for _ in range(NB)]
                       + [pltpu.VMEM((BROWS + 8, 256), U32) for _ in range(NBB)]
                       + [pltpu.VMEM((NP * HD + 8, 128), F32) for _ in range(2)],
        compiler_params=pltpu.CompilerParams(dimension_semantics=("arbitrary",),
                                             vmem_limit_bytes=100 * 1024 * 1024,
                                             disable_bounds_checks=True),
    )(qT, kT, vT)
    return jnp.swapaxes(oT.reshape(B, H, D, S), 2, 3)
```

```python
import bisect
import math

import jax
import jax.numpy as jnp
import jax.experimental.pallas as pl
import jax.experimental.pallas.tpu as pltpu

F32 = jnp.float32
BF16 = jnp.bfloat16
U32 = jnp.uint32

S = 2048
HD = 96
D = 2 * HD
W = 128
N = 4
HS = S // 2
NT = S // W
NS = NT // N
KB = S // N
NG = KB // 128
NB, NBB = 16, 4
NSTATE = 12
KEYS = ('m', 'e', 'M', 'l')

LAM = [1.0 / math.tan(math.pi * (i + 1) / (N + 1)) for i in range(N)]
PAIRS = [(i, j) for i in range(N) for j in range(i + 1, N)]
PRODS = []
for _i in range(N):
    for _j in range(_i + 1, N):
        PRODS += [('s', _i, _j), ('x', _i, _j), ('y', _i, _j)]
    PRODS += [('e', _i, _i), ('f', _i, _i)]
NP = len(PRODS)
PIDX = {p: k for k, p in enumerate(PRODS)}
SUBS = [('d', 0, 2), ('p', 0, 2), ('d', 1, 3), ('p', 1, 3), ('p', 0, 1), ('p', 0, 3), ('p', 1, 2), ('p', 2, 3)]
NSUB = len(SUBS)


def _sgn(i, j):
    return 1.0 if (i + j) % 2 == 1 else -1.0


CH = 208
GV = 4
SIZES = [CH] * (HS // CH) + [HS % CH]
NCH = len(SIZES)
OFFS = [sum(SIZES[:i]) for i in range(NCH)]
GPT = NP * NG
TOT = (3 * HS * NT + NS * GPT * HD) // 4
PER = TOT / NS
NPC = 2 * NSUB
NCL = (KB // 16) * NPC
NGVS = [-(-(sz // 8) // GV) for sz in SIZES]
GOFF = [sum(NGVS[:i]) for i in range(NCH)]
NGV = sum(NGVS)
EG = 4
NEC = -(-NGV // EG)
NCC = N * (HD // 8)
KPIECES = 8
VSUB = len(PAIRS) + N
NV = NG * (HD // 8) * VSUB
QA = 384
PV0, PVN, PVN2 = 15, 10, 36


def _plan(m_ql=250, m_lp=200, m_pm=600, tail=325, espan=400, m_c=250, cspan=5200,
          kt=(600, 6000), vt=(1000, 16000), ww=0.5, alpha=0.15):
    lead_p = PER + m_pm
    lead_q = lead_p + PER + m_lp + espan + m_ql
    span = TOT - tail
    lp = int(math.ceil(lead_p / PER * NCL / NPC)) * NPC
    lq = int(math.ceil(lead_q / (PER / N) * NCH)) + 1
    nm = NS * GPT
    order, load = [], [0, 0, 0, 0]

    def put(n):
        u = min(range(4), key=lambda u: load[u])
        load[u] += n
        return load[u] - n

    mi = rows = 0
    for k in range(NT * NCH):
        sz = SIZES[(k + lq) % NCH]
        order.append(('q', k, max(put(sz) for _ in range(3)), sz))
        rows += sz
        while mi < nm and min(load) + HD // 2 <= sorted(load)[1]:
            order.append(('m', mi, put(HD), HD)); mi += 1
        while mi + 4 <= rows * nm / (NT * HS) + 2 and mi + 4 <= nm:
            for _ in range(4):
                order.append(('m', mi, put(HD), HD)); mi += 1
    while mi < nm:
        order.append(('m', mi, put(HD), HD)); mi += 1

    wts, cnt = [], {}
    for kd, i, j in SUBS:
        if kd == 'd':
            cnt[i] = cnt[j] = 1
            wts += [6.0, 6.0]
        else:
            cnt[i] += 1
            cnt[j] += 1
            extra = sum({N // 2: 1.5, N: 3.0}.get(cnt[q], 0.0) for q in (i, j))
            wts += [12.0 + extra, 16.0 + extra]
    wts = [(1 - ww) + ww * w * len(wts) / sum(wts) for w in wts]
    cap = [1.0] * (TOT // 8 + 64)
    for kd, _, s0, sz in order:
        if kd == 'q':
            cap[s0 // 8:(s0 + sz) // 8] = [1.0 - alpha] * (sz // 8)
    cum = [0.0]
    for t in range(span // 8):
        cum.append(cum[-1] + cap[t])
    tasks, w0 = [], 0.75
    for i in range(NCL * NS):
        y = w0 / (NCL * NS) * cum[-1]
        k = min(bisect.bisect_right(cum, y) - 1, len(cum) - 2)
        tasks.append((8 * (k + (y - cum[k]) / cap[k]), 'p', i + lp))
        w0 += wts[i % NPC]
    for kd, idx, s0, sz in order:
        if kd == 'q' and (idx + lq) % NCH == NCH - 1:
            n = (idx + lq) // NCH
            for u in range(NEC):
                t = s0 + sz + m_ql + u * espan / NEC
                tasks.append((t - span, 'e', (n - NT) * NEC + u) if t >= span else (t, 'e', n * NEC + u))
    le = min(ti for _, kd, ti in tasks if kd == 'e')
    tasks += [(T * PER + m_c + u * cspan / NCC, 'c', T * NCC + u) for T in range(NS) for u in range(NCC)]
    tasks += [(kt[0] + i * (kt[1] - kt[0]) / KPIECES, 'k', i) for i in range(KPIECES)]
    tasks += [(vt[0] + i * (vt[1] - vt[0]) / NV, 'v', i) for i in range(NV)]
    tasks.sort()

    cands = sorted((s + 8 * i, pos, i) for pos, (_, _, s, sz) in enumerate(order) for i in range(sz // 8))
    times = [c[0] for c in cands]
    after, cur = [[] for _ in order], 0
    for t, kd, idx in tasks:
        i = min(bisect.bisect_left(times, t), len(cands) - 1)
        _, pos, vr = min(cands[i:i + 4], key=lambda c: (order[c[1]][0] != 'm', c[1]))
        cur = max(cur, pos)
        after[cur].append((kd, idx, pos, vr))
    return order, after, lq, le, lp


ORDER, AFTER, LQ, LE, LP = _plan()
BROWS = (NP // 2) * (KB // 2)
ASZ = NP * (NG // 2) * (HD // 2)
LSZ = HS // 2


def _live_keys(n):
    qdone = max(0, min(NCH, LQ - n * NCH))
    edone = max(0, min(NEC, LE - n * NEC))
    pdone = max(0, min(NCL, LP - (n // N) * NCL))
    ks = []
    if qdone > 0 and edone < NEC: ks.append('m')
    if 0 < edone < NEC: ks.append('e')
    if edone == NEC and pdone < NCL: ks.append('M')
    if pdone > 0: ks.append('l')
    return ks


def _gate(x, *ms):
    cnd = x > jnp.inf
    return [jnp.where(cnd, x, m) for m in ms]


def _kernel(q_hbm, k_hbm, v_hbm, o_hbm, ibuf, obuf, z_ref, Lc, Ln, Ac, An, Qc, VF, st_scr, isem, osem, *rest):
    S_refs, B_refs, R_refs = rest[:NB], rest[NB:NB + NBB], rest[NB + NBB:]
    NH = q_hbm.shape[0]
    scale = (D ** -0.5) * math.log2(math.e)
    g = pl.program_id(0)

    def in_copy(i, head, par, sem):
        return pltpu.make_async_copy((q_hbm, k_hbm, v_hbm)[i].at[head], ibuf.at[par, i], isem.at[sem])

    def prefetch(par):
        head = jnp.minimum(g + 1, NH - 1)
        for i in range(3):
            in_copy(i, head, par, 0).start()

    def wait_inputs(par):
        pltpu.make_async_copy(ibuf.at[par], ibuf.at[par], isem.at[0]).wait()

    def out_copy(step, piece=None):
        if piece is None:
            return pltpu.make_async_copy(obuf.at[step % 2], o_hbm.at[step - 1], osem.at[0])
        cols = pl.ds(piece * N * W, N * W) if piece < NS - 1 else pl.ds((piece + (NS - 1) * (N - 1)) * W, W)
        return pltpu.make_async_copy(obuf.at[step % 2, :, cols], o_hbm.at[step - 1, :, cols], osem.at[1 + piece])

    def body(first, last):
        z = z_ref[0]
        fence = lambda r: pl.ds(pl.multiple_of(r + z * 8, 8), 8)
        par = 0 if first else g % 2
        q_next, k_next, v_next = [ibuf.at[par, i] for i in range(3)]
        st = [dict() for _ in range(NT + NSTATE)]
        acc, res = {}, {}
        done = dict(k=0, q=set(), p=set(), m=set(), c=set())

        def kprep(c0, c1):
            a1, a2, a3 = [k_next[r:r + 64, c0:c1] for r in (0, 64, 128)]
            b1, b2, b3 = [k_next[r:r + 64, HS + c0:HS + c1] for r in (0, 64, 128)]
            d1 = (a2.astype(F32) - b2.astype(F32)).astype(BF16)
            d2 = (b1.astype(F32) - a1.astype(F32)).astype(BF16)
            for i, (x, y) in enumerate(((a1, b2), (d1, a3), (d2, b3))):
                Ln[i * LSZ + c0 // 2:i * LSZ + c1 // 2, :] = pltpu.bitcast(
                    jnp.concatenate([x, y], axis=0).T, U32)

        def vprep(sb, xs):
            x = jnp.concatenate([jnp.concatenate(xs[r::HD // 8], axis=1) for r in range(HD // 8)], axis=0)
            ldf = lambda half, kb: v_next[half * HD:(half + 1) * HD, kb * KB:(kb + 1) * KB].astype(F32)

            def put_a(p, u):
                for jp in range(NG // 2):
                    ao = (PIDX[p] * (NG // 2) + jp) * (HD // 2)
                    An[ao:ao + HD // 2, :] = pltpu.bitcast(u[:, jp * 256:(jp + 1) * 256].astype(BF16), U32)

            if sb < N:
                a1, = _gate(x, ldf(0, sb))
                fi = LAM[sb] * a1 + ldf(1, sb)
                put_a(('e', sb, sb), a1)
                put_a(('f', sb, sb), fi)
                VF[sb * HD:(sb + 1) * HD, :] = fi
                if sb == N - 1:
                    VF[fence(N * HD), 0:W] = xs[-1]
            else:
                i, jj = PAIRS[sb - N]
                fi, = _gate(x, VF[i * HD:(i + 1) * HD, :])
                fj = VF[jj * HD:(jj + 1) * HD, :]
                s = (fi + fj if _sgn(i, jj) > 0 else fi - fj) * (1.0 / (LAM[i] - LAM[jj]))
                s = pltpu.bitcast((pltpu.bitcast(s, U32) + 0x8000) & jnp.uint32(0xFFFF0000), F32)
                put_a(('s', i, jj), s)
                put_a(('x', i, jj), s - ldf(0, i))
                put_a(('y', i, jj), s + ldf(0, jj) if _sgn(i, jj) > 0 else s - ldf(0, jj))

        def qcopy(n):
            Qc[n * HD:(n + 1) * HD, :] = pltpu.bitcast(q_next[:, n * W:(n + 1) * W], U32)

        def qk(n, ci):
            t, nxt = st[n], n >= NT
            assert first or n < NB or (n - NB) // N in done['p']
            if nxt:
                assert first or done['k'] == KPIECES
                if 'q' not in t:
                    t['q'] = q_next[:, (n - NT) * W:(n - NT + 1) * W]
                q = t['q']
            else:
                q = pltpu.bitcast(Qc[n * HD:(n + 1) * HD, :], BF16)
            r0, rows = OFFS[ci], SIZES[ci]
            Lr = Ln if nxt or last else Lc
            lhs = lambda i: pltpu.bitcast(Lr[i * LSZ + r0 // 2:i * LSZ + (r0 + rows) // 2, :], BF16)
            p3 = jnp.dot(lhs(0), q[0:128], preferred_element_type=F32)
            p1 = jnp.dot(lhs(1), q[64:192], preferred_element_type=F32)
            p2 = jnp.dot(lhs(2), jnp.concatenate([q[0:64], q[128:192]], axis=0), preferred_element_type=F32)
            sa = (p1 + p3) * scale
            sb = (p2 + p3) * scale
            Sr = S_refs[n % NB]
            Sr[r0:r0 + rows, :] = sa
            Sr[HS + r0:HS + r0 + rows, :] = sb
            sab = jnp.maximum(sa, sb).reshape(rows // 8, 8, W)
            for gi in range(NGVS[ci]):
                gm = sab[gi * GV:(gi + 1) * GV].max(axis=0)
                go = S + 8 + (GOFF[ci] + gi) * 8
                Sr[go:go + 8, :] = gm
                t['m'] = jnp.maximum(t['m'], gm) if 'm' in t else gm
            if ci == NCH - 1:
                t['m'] = jnp.broadcast_to(jnp.max(t['m'], axis=0, keepdims=True), (8, W))
                Sr[fence(S), :] = t['m']
                done['q'].add(n)
                if not nxt and not last:
                    qcopy(n)
            return p3

        def ecl(idx, x):
            n, u = divmod(idx, NEC)
            assert n in done['q']
            t = st[n]
            g0, g1 = u * EG, min(NGV, u * EG + EG)
            s = S_refs[n % NB][S + 8 + g0 * 8:S + 8 + g1 * 8, :].reshape(g1 - g0, 8, W)
            m, = _gate(x, t['m'])
            e = jnp.exp2(s - m[None]).sum(axis=0)
            t['e'] = t['e'] + e if 'e' in t else e
            if u == NEC - 1:
                tot = jnp.sum(t.pop('e'), axis=0, keepdims=True)
                t['M'] = t.pop('m') + jnp.broadcast_to(jnp.log2(tot), (8, W))

        def pstage(T, s0, s1, xs):
            ns = s1 - s0
            Br = B_refs[T % NBB]
            assert first or T < NBB or (T - NBB) in done['m']

            def put_b(p, v):
                off, cb = (PIDX[p] // 2) * (KB // 2), (PIDX[p] % 2) * W
                Br[off + 8 * s0:off + 8 * s1, cb:cb + W] = pltpu.bitcast(v.reshape(16 * ns, W).astype(BF16), U32)

            rs, cs, cnt, ev = {}, {}, {}, {}
            for sb, (kd, i, j) in enumerate(SUBS):
                Ms = {q: _gate(jnp.stack(xs[2 * sb + hh::NPC]), st[N * T + q]['M'][None])[0]
                      for hh, q in enumerate((j, i))}

                def b(kb, q):
                    s = S_refs[(N * T + q) % NB][kb * KB + 16 * s0:kb * KB + 16 * s1, :].reshape(ns, 2, 8, W)
                    return jnp.exp2(s - Ms[q][:, None])

                if kd == 'd':
                    for q in (i, j):
                        rs[q] = cs[q] = b(q, q)
                        cnt[q] = 1
                else:
                    bij, bji = b(i, j), b(j, i)
                    upd = (lambda a, v: a - v) if _sgn(i, j) > 0 else (lambda a, v: a + v)
                    put_b(('x', i, j), bij)
                    put_b(('y', i, j), bji)
                    put_b(('s', i, j), bij - bji)
                    rs[i], rs[j] = upd(rs[i], bij), upd(rs[j], bji)
                    cs[i], cs[j] = upd(cs[i], bji), upd(cs[j], bij)
                    cnt[i] += 1
                    cnt[j] += 1
                for q in (i, j):
                    if cnt[q] == N // 2:
                        ev[q] = cs[q][:, 0] + cs[q][:, 1]
                        ev[q] = ev[q] + ev[q]
                    if cnt[q] == N:
                        put_b(('e', q, q), rs[q])
                        put_b(('f', q, q), cs[q])
            for q in range(N):
                t = st[N * T + q]
                od = cs[q][:, 0] + cs[q][:, 1]
                for s in range(ns):
                    t['l'] = (t['l'] + ev[q][s] if 'l' in t else ev[q][s]) - od[s]
            if s1 == KB // 16:
                Br[fence(BROWS), 0:W] = pltpu.bitcast(st[N * T]['M'], U32)
                for q in range(N):
                    t = st[N * T + q]
                    del t['M']
                    t['l'] = jnp.broadcast_to(1.0 / jnp.sum(t['l'], axis=0, keepdims=True), (8, W))
                done['p'].add(T)

        def mgroup(gi):
            T, r = divmod(gi, GPT)
            pi, j = divmod(r, NG)
            assert T in done['p'] and (j > 0 or T < 1 or (T - 2) in done['c'])
            ao = ((pi * NG + j) // 2) * (HD // 2)
            if last:
                a = An[ao:ao + HD // 2, (j % 2) * W:(j % 2 + 1) * W]
            else:
                a = Ac[(j % 2) * ASZ + ao:(j % 2) * ASZ + ao + HD // 2, :]
            bo = (pi // 2) * (KB // 2) + j * 64
            b = B_refs[T % NBB][bo:bo + 64, (pi % 2) * W:(pi % 2 + 1) * W]
            oj = jnp.dot(pltpu.bitcast(a, BF16), pltpu.bitcast(b, BF16), preferred_element_type=F32)
            acc['o'] = oj if j == 0 else acc['o'] + oj
            if j == NG - 1:
                R_refs[T % 2][pi * HD:(pi + 1) * HD, :] = acc.pop('o')
                inline = last and T == NS - 1
                if pi == NP - 1:
                    done['m'].add(T)
                    if not inline:
                        R_refs[T % 2][fence(NP * HD), :] = oj[0:8]
                if inline and PRODS[pi][0] == 'f':
                    combine(T, PRODS[pi][1], oj)
            return oj

        def combine(T, q, x):
            assert T < 0 or T in done['m'] or (last and T == NS - 1)
            R = lambda *p: R_refs[T % 2][PIDX[p] * HD:(PIDX[p] + 1) * HD, :]
            add = lambda a, sg, v: a + v if sg > 0 else a - v
            others = ([(i, -1.0, R('x', i, q)) for i in range(q)]
                      + [(jj, _sgn(q, jj), R('y', q, jj)) for jj in range(q + 1, N)])
            gq, = _gate(x, R('e', q, q))
            for jj in range(q + 1, N):
                gq = add(add(gq, _sgn(q, jj), R('s', q, jj)), -_sgn(q, jj), R('x', q, jj))
            for i in range(q):
                gq = (gq + R('y', i, q)) + R('s', i, q)
            c1 = gq
            c2 = R('f', q, q) - LAM[q] * gq
            for t_, sg, v in others:
                c1 = add(c1, sg, v)
                c2 = c2 - (sg * LAM[t_]) * v
            if T < 0:
                linv, ob = st_scr[NSTATE * 4 + q], obuf.at[(g - 1) % 2]
            else:
                linv, ob = st[N * T + q]['l'], obuf.at[g % 2]
            q0 = (N * (T % NS) + q) * W
            for half, cc in enumerate((c1, c2)):
                cc = (cc.reshape(HD // 8, 8, W) * linv[None]).reshape(HD, W)
                ob[half * HD:(half + 1) * HD, q0:q0 + W] = cc.astype(ob.dtype)
            if q == N - 1:
                done['c'].add(T)
                if T < 0:
                    @pl.when(g > 1)
                    def _():
                        out_copy(g - 1).start()
                elif last and T < NS - 1:
                    out_copy(g, T).start()
            if last and T == NS - 1:
                out_copy(g, T + q).start()

        pend = dict(p=[], c=[], v=[])

        def flush_p(ti):
            T, k = divmod(ti, NCL)
            s1 = k // NPC + 1
            pstage(T, s1 - len(pend['p']) // NPC, s1, pend['p'])
            pend['p'] = []

        def pcl(ti, x):
            pend['p'].append(x)
            pend['pi'] = ti
            if ti % NCL == NCL - 1:
                flush_p(ti)

        def ccl(ti, x):
            pend['c'].append(x)
            if len(pend['c']) == HD // 8:
                T, u = divmod(ti, NCC)
                combine(T - 1, u // (HD // 8), jnp.concatenate(pend['c'], axis=0))
                pend['c'] = []

        def vcl(ti, x):
            pend['v'].append(x)
            if len(pend['v']) == NV // VSUB:
                vprep(ti // (NV // VSUB), pend['v'])
                pend['v'] = []

        if first:
            qa = pltpu.make_async_copy(q_hbm.at[0, :, 0:QA], ibuf.at[0, 0, :, 0:QA], isem.at[1])
            qb = pltpu.make_async_copy(q_hbm.at[0, :, QA:S], ibuf.at[0, 0, :, QA:S], isem.at[4])
            in_copy(1, 0, 0, 2).start()
            qa.start()
            in_copy(2, 0, 0, 3).start()
            qb.start()
            R_refs[(NS - 1) % 2][0:NP * HD, :] = jnp.zeros((NP * HD, W), F32)
            for q in range(N):
                st_scr[NSTATE * 4 + q] = jnp.zeros((8, W), F32)
            in_copy(1, 0, 0, 2).wait()
            qa.wait()
            kprep(0, HS)
        else:
            if not last:
                Lc[0:3 * LSZ, :] = Ln[0:3 * LSZ, :]
                for i in range(2):
                    Ac[i * ASZ:(i + 1) * ASZ, :] = An[0:ASZ, i * W:(i + 1) * W]
            for n in range(NSTATE):
                for key in _live_keys(n):
                    st[n][key] = st_scr[n * 4 + KEYS.index(key)]
                if LQ >= (n + 1) * NCH: done['q'].add(n)
                if LP >= (n // N + 1) * NCL: done['p'].add(n // N)

        pw = HS // KPIECES
        run = dict(e=ecl, p=pcl, c=ccl, v=vcl)

        def active(pos):
            kd, idx = ORDER[pos][0:2]
            if kd == 'm': return not first
            n = (idx + LQ) // NCH
            return (not first or n >= NT) and (not last or n < NT)

        def wanted(tk, ti):
            lim = NCL * NS if tk == 'p' else NT * NEC
            if first: return tk not in 'kvc' and ti >= lim
            if last: return tk == 'c' or (tk not in 'kv' and ti < lim)
            return True

        acts = [pos for pos in range(len(ORDER)) if active(pos)]
        nq, vdone = 0, 0
        for ai, pos in enumerate(acts):
            kd, idx = ORDER[pos][0:2]
            res[pos] = qk(*divmod(idx + LQ, NCH)) if kd == 'q' else mgroup(idx)
            end = acts[ai + 1] if ai + 1 < len(acts) else len(ORDER)
            todo = [t for p2 in range(pos, end) for t in AFTER[p2] if wanted(t[0], t[1])]
            if first:
                nq += 1
                if nq == PV0:
                    assert nq <= (QA // W) * NCH
                    in_copy(2, 0, 0, 3).wait()
                    qb.wait()
                    prefetch(1)
                if nq == PV0 + 1:
                    for n2 in range(LQ // NCH, NT):
                        qcopy(n2)
                if nq > PV0:
                    nv = min(NV - vdone, PVN if any(t[0] == 'p' for t in todo) else PVN2)
                    vs = [('v', vdone + u, None, 0) for u in range(nv)]
                    vdone += nv
                    mix = sorted([((i + 0.5) / len(todo), t) for i, t in enumerate(todo)]
                                 + [((i + 0.25) / nv, t) for i, t in enumerate(vs)], key=lambda a: a[0])
                    todo = [t for _, t in mix]
            nvr = res[pos].shape[0] // 8
            for i, (tk, ti, tpos, vr) in enumerate(todo):
                if first or tpos not in res:
                    tpos, vr = pos, (i * nvr) // len(todo)
                x = res[tpos][8 * vr:8 * vr + 8]
                if tk == 'k':
                    kprep(ti * pw, (ti + 1) * pw)
                    done['k'] += 1
                else:
                    run[tk](ti, x)
        if pend['p']:
            flush_p(pend['pi'])
        assert not pend['c'] and (not first or vdone == NV)
        if not last:
            if not first:
                for q in range(N):
                    st_scr[NSTATE * 4 + q] = st[NT - N + q]['l']
            for n in range(NSTATE):
                assert sorted(k for k in st[NT + n] if k != 'q') == sorted(_live_keys(n))
                for key in _live_keys(n):
                    st_scr[n * 4 + KEYS.index(key)] = st[NT + n][key]

    def step(last):
        if not last:
            prefetch((g + 1) % 2)
        body(False, last)
        if not last:
            wait_inputs((g + 1) % 2)

        @pl.when(g > 1)
        def _():
            out_copy(g - 1).wait()

        if last:
            for piece in range(NS + N - 1):
                out_copy(g, piece).wait()

    @pl.when(g == 0)
    def _():
        z_ref[0] = 0
        body(True, False)
        wait_inputs(1)

    @pl.when(jnp.logical_and(g > 0, g < NH))
    def _():
        step(False)

    @pl.when(g == NH)
    def _():
        step(True)


@jax.jit
def pallas_standalone__mha_softmax__prompt_kernel(q: jax.Array, k: jax.Array, v: jax.Array):
    B, H, sq, d = q.shape
    assert sq == S and d == D and k.shape == q.shape and v.shape == q.shape
    NH = B * H
    qT, kT, vT = [jnp.swapaxes(x, 2, 3).reshape(NH, D, S) for x in (q, k, v)]
    oT = pl.pallas_call(
        _kernel,
        grid=(NH + 1,),
        in_specs=[pl.BlockSpec(memory_space=pl.ANY)] * 3,
        out_specs=pl.BlockSpec(memory_space=pl.ANY),
        out_shape=jax.ShapeDtypeStruct((NH, D, S), q.dtype),
        scratch_shapes=[pltpu.VMEM((2, 3, D, S), q.dtype), pltpu.VMEM((2, D, S), q.dtype),
                        pltpu.SMEM((1,), jnp.int32),
                        pltpu.VMEM((3 * LSZ + 128, 128), U32), pltpu.VMEM((3 * LSZ + 128, 128), U32),
                        pltpu.VMEM((2 * ASZ + 128, 128), U32), pltpu.VMEM((ASZ + 64, 256), U32),
                        pltpu.VMEM((NT * HD + 128, 128), U32), pltpu.VMEM((N * HD + 64, KB), F32),
                        pltpu.VMEM((NSTATE * 4 + 16, 8, 128), F32),
                        pltpu.SemaphoreType.DMA((5,)), pltpu.SemaphoreType.DMA((NS + N,))]
                       + [pltpu.VMEM((S + 8 + 8 * NGV, W), F32) for _ in range(NB)]
                       + [pltpu.VMEM((BROWS + 8, 256), U32) for _ in range(NBB)]
                       + [pltpu.VMEM((NP * HD + 8, 128), F32) for _ in range(2)],
        compiler_params=pltpu.CompilerParams(dimension_semantics=("arbitrary",),
                                             vmem_limit_bytes=100 * 1024 * 1024,
                                             disable_bounds_checks=True),
    )(qT, kT, vT)
    return jnp.swapaxes(oT.reshape(B, H, D, S), 2, 3)
```
